```python
import jax
import jax.numpy as jnp

def _softmax(x, axis=-1):
    return jax.nn.softmax(x, axis=axis)

def _gelu(x):
    return jax.nn.gelu(x, approximate=True)

def _silu(x):
    return jax.nn.silu(x)

def _sigmoid(x):
    return jax.nn.sigmoid(x)

def _layernorm(x, axis=-1, eps=1e-05):
    m = jnp.mean(x, axis=axis, keepdims=True)
    v = jnp.var(x, axis=axis, keepdims=True)
    return (x - m) / jnp.sqrt(v + eps)

def _scatter_add(tgt, idx, src, axis=0):
    return tgt.at[idx].add(src)

def _segment_sum(src, seg, n):
    return jax.ops.segment_sum(src, seg, n)

class _Rng:

    def __init__(self, key):
        self._k = key

    def _next(self):
        self._k, sub = jax.random.split(self._k)
        return sub

    def normal(self, shape):
        return jax.random.normal(self._next(), shape, dtype=jnp.bfloat16)

    def randint(self, lo, hi, shape):
        return jax.random.randint(self._next(), shape, lo, hi, dtype=jnp.int32)

    def uniform(self, shape, lo=0.0, hi=1.0):
        return jax.random.uniform(self._next(), shape, jnp.bfloat16, lo, hi)

    def permutation(self, n):
        return jax.random.permutation(self._next(), n)
kernel_name = 'sequential_preLN__memory_aug_infini_attn__moe_arch_mod__prompt'

def setup_inputs():
    _rng = _Rng(jax.random.key(int.from_bytes(__import__("os").urandom(4), "little")))
    _w = lambda a: (lambda t: t.astype(jnp.bfloat16) if jnp.issubdtype(t.dtype, jnp.floating) else t)(jnp.asarray(a))

    def _A_setup():
        B, S, D, H = (1, 2048, 576, 32)
        N = 4
        L = max(1, S // N)
        sc = D ** (-0.5)
        return {'x': _w((lambda *s: _rng.normal(s) * 0.05)(B, N * L, D)), 'wq': _w((lambda *s: _rng.normal(s) * 0.05)(D, D) * sc), 'wk': _w((lambda *s: _rng.normal(s) * 0.05)(D, D) * sc), 'wv': _w((lambda *s: _rng.normal(s) * 0.05)(D, D) * sc), 'wo': _w((lambda *s: _rng.normal(s) * 0.05)(D, D) * sc), 'beta': _w((lambda *s: _rng.normal(s) * 0.05)(H))}
    _A_in = _A_setup()

    def _B_setup():
        B, S, D, F, C = (1, 2048, 576, 4608, 1)
        return {'x': _w((lambda *s: _rng.normal(s) * 0.05)(B, S, D)), 'w_r': _w((lambda *s: _rng.normal(s) * 0.05)(D)), 'w_gate': _w((lambda *s: _rng.normal(s) * 0.05)(D, F)), 'w_up': _w((lambda *s: _rng.normal(s) * 0.05)(D, F)), 'w_down': _w((lambda *s: _rng.normal(s) * 0.05)(F, D))}
    _B_in = _B_setup()
    return {'A_x': _A_in['x'], 'A_wq': _A_in['wq'], 'A_wk': _A_in['wk'], 'A_wv': _A_in['wv'], 'A_wo': _A_in['wo'], 'A_beta': _A_in['beta'], 'B_x': _B_in['x'], 'B_w_r': _B_in['w_r'], 'B_w_gate': _B_in['w_gate'], 'B_w_up': _B_in['w_up'], 'B_w_down': _B_in['w_down']}

def reference(A_x, A_wq, A_wk, A_wv, A_wo, A_beta, B_x, B_w_r, B_w_gate, B_w_up, B_w_down):

    def _A_ref(x, wq, wk, wv, wo, beta):
        B, S, D = x.shape
        H = 32
        Dh = D // H
        N = 4
        L = S // N
        q = (lambda x, *d: x.transpose(*d))((x @ wq).reshape(B, S, H, Dh), 0, 2, 1, 3).reshape(B, H, N, L, Dh)
        k = (lambda x, *d: x.transpose(*d))((x @ wk).reshape(B, S, H, Dh), 0, 2, 1, 3).reshape(B, H, N, L, Dh)
        v = (lambda x, *d: x.transpose(*d))((x @ wv).reshape(B, S, H, Dh), 0, 2, 1, 3).reshape(B, H, N, L, Dh)
        phi = lambda t: jnp.where(t > 0, t + 1.0, jnp.exp(t))
        scale = Dh ** (-0.5)
        ar = jnp.arange(L)
        mask = (lambda x, dt: x.astype(dt))(ar[:, None] < ar[None, :], x.dtype) * -1000000000.0
        g = _sigmoid(beta).reshape(1, H, 1, 1)
        M = jnp.einsum('bhd,bhe->bhde', q[:, :, 0, 0, :] * 0.0, q[:, :, 0, 0, :] * 0.0)
        z = q[:, :, 0, 0, :] * 0.0
        outs = []
        for s in range(N):
            qs, ks, vs = (q[:, :, s].copy(), k[:, :, s].copy(), v[:, :, s].copy())
            logits = jnp.einsum('bhqd,bhkd->bhqk', qs, ks) * scale + mask
            p = _softmax(logits, axis=-1)
            a_dot = jnp.einsum('bhqk,bhkd->bhqd', p, vs)
            pq = phi(qs)
            num = jnp.einsum('bhld,bhde->bhle', pq, M)
            den = jnp.einsum('bhld,bhd->bhl', pq, z)[..., None] + 1e-06
            a_mem = num / den
            o = g * a_mem + (1.0 - g) * a_dot
            outs.append(o)
            pk = phi(ks)
            M = M + jnp.einsum('bhld,bhle->bhde', pk, vs)
            z = z + jnp.einsum('bhld->bhd', pk)
        o = (lambda x, *d: x.transpose(*d))(jnp.stack(outs, 2).reshape(B, H, S, Dh), 0, 2, 1, 3).reshape(B, S, D)
        return o @ wo

    def _B_ref(x, w_r, w_gate, w_up, w_down):
        B, S, D = x.shape
        C = 1
        r = x @ w_r
        idx = jnp.argsort(-r, axis=-1)[:, :C]
        idx_e = jnp.repeat(idx.reshape(B, C, 1), D, axis=2)
        x_sel = jnp.take_along_axis(x, idx_e, axis=1)
        g = _silu(x_sel @ w_gate)
        u = x_sel @ w_up
        y = g * u @ w_down
        r_sel = _sigmoid(jnp.take_along_axis(r, idx, axis=1))
        y = y * r_sel.reshape(B, C, 1)
        b_off = (jnp.arange(B) * S).reshape(B, 1)
        flat_idx = (idx + b_off).reshape(B * C)
        zero = (x * 0.0).reshape(B * S, D)
        upd = _scatter_add(zero, flat_idx, y.reshape(B * C, D), axis=0)
        return x + upd.reshape(B, S, D)
    x = A_x
    h = x + _A_ref(_layernorm(x, axis=-1), A_wq, A_wk, A_wv, A_wo, A_beta)
    h2 = h + _B_ref(_layernorm(h, axis=-1), B_w_r, B_w_gate, B_w_up, B_w_down)
    return h2
```

```python
import functools

import jax
import jax.numpy as jnp
import numpy as np
from jax import lax
import jax.experimental.pallas as pl
import jax.experimental.pallas.tpu as pltpu

F32 = jnp.float32
BF16 = jnp.bfloat16
I32 = jnp.int32

SEQ = 2048
D = 576
DP = 640
H = 32
DH = 18
NSEG = 4
L = 512
FF = 4608
NG = 5
HPG = 7
LAST_ROWS = 80
QV_ROWS = 4 * 128 + LAST_ROWS
EPS = 1e-05
LOG2E = 1.4426950408889634
QSCALE = float(DH ** -0.5) * LOG2E
SAFE_BOUND = 40.0
V_BOUND = 2.0 ** 40
MROWS = 144


def _heads_in(g):
    return min(HPG, H - HPG * g)


def _iota(shape, dim):
    return lax.broadcasted_iota(I32, shape, dim)


def _ln(xf, axis=0):
    m = jnp.mean(xf, axis=axis, keepdims=True)
    xc = xf - m
    v = jnp.mean(xc * xc, axis=axis, keepdims=True)
    return xc * lax.rsqrt(v + EPS)


def _phi(t):
    return jnp.where(t > 0, t + 1.0, jnp.exp(t))


def _kernel(x_hbm, wq_hbm, wk_hbm, wv_hbm, wo_hbm, beta_hbm, wr_hbm,
            wg_hbm, wu_hbm, wd_hbm, out_hbm,
            x_v, wraw, wtmp, wT, woT, wg_v, wu_v, wd_v, beta_v, wr_v, wr_col,
            k_g, pkT_g, qT_g, pqT_g, vT_g, p_buf, oT, am, MT, grep, omg,
            h_v, h2_v, patch_v, oslow, rb_ref, ib_ref,
            sem_x, sem_w, sem_f, sem_o, sem_p, sem_s):
    def x_copy(s):
        return pltpu.make_async_copy(x_hbm.at[:, pl.ds(s * L, L)], x_v.at[s], sem_x.at[s])

    def w_copy(i):
        src = (wq_hbm, wk_hbm, wv_hbm, wo_hbm)[i]
        return pltpu.make_async_copy(src, wraw.at[i, pl.ds(0, D), :], sem_w.at[i])

    def s_copy(i):
        src, dst = ((beta_hbm, beta_v), (wr_hbm, wr_v))[i]
        return pltpu.make_async_copy(src, dst, sem_s.at[i])

    def f_copy(i):
        src, dst = ((wg_hbm, wg_v), (wu_hbm, wu_v), (wd_hbm, wd_v))[i]
        return pltpu.make_async_copy(src, dst, sem_f.at[i])

    def o_copy(s):
        return pltpu.make_async_copy(h2_v.at[s], out_hbm.at[:, pl.ds(s * L, L)], sem_o.at[s])

    wraw[:, pl.ds(D, DP - D), :] = jnp.zeros((4, DP - D, D), BF16)
    w_copy(0).start()
    x_copy(0).start()
    w_copy(1).start()
    w_copy(2).start()
    s_copy(0).start()
    s_copy(1).start()
    w_copy(3).start()

    MT[...] = jnp.zeros(MT.shape, F32)
    qT_g[NG - 1] = jnp.zeros((128, L), BF16)
    pqT_g[NG - 1] = jnp.zeros((128, L), BF16)
    pkT_g[NG - 1] = jnp.zeros((128, L), BF16)
    vT_g[NG - 1] = jnp.zeros((128, L), BF16)
    rb_ref[...] = jnp.full((8, L), -jnp.inf, F32)
    ib_ref[...] = jnp.zeros((8, L), I32)

    def windows(src, dst, rows):
        keep = _iota((rows, 128), 1) < HPG * DH
        for g in range(NG - 1):
            w = src[0:rows, HPG * DH * g: HPG * DH * g + 128]
            dst[0:rows, 128 * g: 128 * (g + 1)] = jnp.where(keep, w, jnp.zeros_like(w))
        dst[0:rows, 512:640] = jnp.zeros((rows, 128), BF16)
        dst[0:rows, 512:512 + 72] = src[0:rows, 504:576]

    for i in range(3):
        w_copy(i).wait()
        windows(wraw.at[i], wtmp, DP)
        wt = wtmp[...].T
        wT[i] = wt[0:QV_ROWS, :]
    w_copy(3).wait()
    wtmp[:, 0:D] = wraw[3]
    wtmp[:, D:DP] = jnp.zeros((DP, DP - D), BF16)
    wraw[0, :, :] = wtmp[...].T[:, 0:D]
    windows(wraw.at[0], woT, D)

    for s in range(1, NSEG):
        x_copy(s).start()
    for i in range(3):
        f_copy(i).start()

    s_copy(0).wait()
    s_copy(1).wait()
    beta = beta_v[...].reshape(1, H).astype(F32)
    gate = jax.nn.sigmoid(beta)
    gate = jnp.concatenate([gate, jnp.zeros((1, 128 - H), F32)], axis=1)
    lane = _iota((128, 128), 1)
    row = _iota((128, 128), 0)
    lane8 = _iota((8, 128), 1)
    row8 = _iota((8, 128), 0)
    for g in range(NG):
        hid = HPG * g + row // DH
        sel = (lane == hid) & (row < _heads_in(g) * DH)
        gcol = jnp.sum(jnp.where(sel, jnp.broadcast_to(gate, (128, 128)), 0.0), axis=1, keepdims=True)
        grep[g] = jnp.broadcast_to(gcol, (128, 128))
        sel8 = (lane8 == HPG * g + row8) & (row8 < _heads_in(g))
        g8 = jnp.sum(jnp.where(sel8, jnp.broadcast_to(gate, (8, 128)), 0.0), axis=1, keepdims=True)
        omg[g] = jnp.broadcast_to(1.0 - g8, (8, 128))
    wr = wr_v[...].reshape(1, D).astype(F32)
    wr = jnp.concatenate([wr, jnp.zeros((1, DP - D), F32)], axis=1)
    wr_col[...] = jnp.broadcast_to(wr, (128, DP)).T

    r128 = _iota((128, 128), 0)
    c128 = _iota((128, 128), 1)
    diag_ok = r128 <= c128
    mrow = _iota((MROWS, 128), 0)
    mlane = _iota((MROWS, 128), 1)
    mhead = jnp.where(mrow < 128, mrow // DH, mrow - 128)
    mmask = (mhead == mlane // DH) & (mlane < HPG * DH) & ((mrow < HPG * DH) | (mrow >= 128))
    ones16 = jnp.ones((16, L), BF16)

    def head_window(j):
        return (DH * j // 16) * 16

    def proj(i, xn):
        return lax.dot_general(wT[i, :, 0:D], xn, (((1,), (0,)), ((), ())),
                               preferred_element_type=F32)

    def seg_body(s, carry):
        x_copy(s).wait()
        xb = x_v[s]
        xn = _ln(xb.astype(F32)).astype(BF16)

        q = proj(0, xn)
        qmax = jnp.max(jnp.abs(q))
        for g in range(NG):
            nr = 128 if g < NG - 1 else LAST_ROWS
            qg = q[128 * g:128 * g + nr]
            qT_g[g, 0:nr, :] = (qg * QSCALE).astype(BF16)
            pqT_g[g, 0:nr, :] = _phi(qg).astype(BF16)
        k = proj(1, xn)
        kmax = jnp.max(jnp.abs(k))
        for g in range(NG):
            nr = 128 if g < NG - 1 else LAST_ROWS
            kg = k[128 * g:128 * g + nr]
            kb = kg.astype(BF16)
            if nr < 128:
                kb = jnp.concatenate([kb, jnp.zeros((128 - nr, L), BF16)], axis=0)
            k_g[g] = kb.T
            pkT_g[g, 0:nr, :] = _phi(kg).astype(BF16)
        v = proj(2, xn)
        vmax = jnp.max(jnp.abs(v))
        for g in range(NG):
            nr = 128 if g < NG - 1 else LAST_ROWS
            vT_g[g, 0:nr, :] = v[128 * g:128 * g + nr].astype(BF16)
        safe = (qmax * kmax * (DH * QSCALE * 1.02) <= SAFE_BOUND) & (vmax <= V_BOUND)

        for g in range(NG):
            _group(g)

        @pl.when(jnp.logical_not(safe))
        def _():
            _slow_attention()

        ot = jnp.concatenate([oT[g] for g in range(NG)], axis=0)
        outT = jnp.dot(woT[...], ot, preferred_element_type=F32)
        hb = (xb.astype(F32) + outT.astype(BF16).astype(F32)).astype(BF16)
        hf = hb.astype(F32)
        hn = _ln(hf).astype(BF16).astype(F32)
        h_v[s] = hb
        h2_v[s] = (hf + hn).astype(BF16)
        o_copy(s).start()
        wc = wr_col[0:D, :]
        r = jnp.concatenate(
            [jnp.sum(hn[:, 128 * t:128 * (t + 1)] * wc, axis=0, keepdims=True) for t in range(4)],
            axis=1)
        r = jnp.broadcast_to(r, (8, L))
        upd = r > rb_ref[...]
        rb_ref[...] = jnp.where(upd, r, rb_ref[...])
        ib_ref[...] = jnp.where(upd, _iota((8, L), 1) + s * L, ib_ref[...])
        return carry

    def _group(g):
        nh = _heads_in(g)
        mt = MT[g]
        gx = jnp.concatenate([grep[g], jnp.ones((MROWS - 128, 128), F32)], axis=0)
        mtb = jnp.where(mmask, mt * gx, 0.0).astype(BF16)
        nd = jnp.dot(mtb, pqT_g[g], preferred_element_type=F32)
        rden = 1.0 / (nd[128:136] + 1e-06)
        for r in range(16):
            lo, hi = 8 * r, 8 * r + 8
            h0, h1 = lo // DH, min((hi - 1) // DH, HPG - 1)
            rd = jnp.broadcast_to(rden[h0:h0 + 1], (8, L))
            if h1 != h0:
                rd = jnp.where(_iota((8, L), 0) + lo < DH * h1, rd,
                               jnp.broadcast_to(rden[h1:h1 + 1], (8, L)))
            am[g, lo:hi, :] = nd[lo:hi] * rd
        lhs = jnp.concatenate([vT_g[g], ones16], axis=0)
        MT[g] = mt + lax.dot_general(lhs, pkT_g[g], (((1,), (1,)), ((), ())),
                                     preferred_element_type=F32)

        def qk(qb, slot):
            nk = (qb + 1) * 128
            qt = pltpu.bitcast(qT_g[g, :, qb * 128:(qb + 1) * 128], I32)
            rr = _iota((64, 128), 0)
            qm = jnp.concatenate(
                [pltpu.bitcast(jnp.where((rr >= 9 * j) & (rr < 9 * j + 9), qt, 0), BF16)
                 for j in range(nh)], axis=1)
            sc = jnp.dot(k_g[g, 0:nk, :], qm, preferred_element_type=F32)
            p = jnp.exp2(sc).astype(BF16)
            if nk > 128:
                p_buf[slot, 0:nk - 128, 0:nh * 128] = p[0:nk - 128]
            for j in range(nh):
                pd = p[nk - 128:nk, j * 128:(j + 1) * 128]
                p_buf[slot, nk - 128:nk, j * 128:(j + 1) * 128] = jnp.where(diag_ok, pd, jnp.zeros_like(pd))

        def pv(qb, slot):
            nk = (qb + 1) * 128
            vals = []
            for j in range(nh):
                a = head_window(j)
                vw = pltpu.bitcast(vT_g[g, a:a + 32, 0:nk], I32)
                vw = jnp.where(_iota((16, nk), 0) == 15, 0x3F803F80, vw)
                acc = jnp.dot(pltpu.bitcast(vw, BF16), p_buf[slot, 0:nk, j * 128:(j + 1) * 128],
                              preferred_element_type=F32)
                rd = omg[g, j:j + 1, :] / acc[31:32]
                vals.append((acc, jnp.broadcast_to(rd, (8, 128))))
            rows = []
            for r in range(16):
                lo, hi = 8 * r, 8 * r + 8
                h0, h1 = lo // DH, (hi - 1) // DH
                val = am[g, lo:hi, qb * 128:(qb + 1) * 128]
                if h0 < nh:
                    a0 = head_window(h0)
                    d = vals[h0][0][lo - a0:hi - a0] * vals[h0][1]
                    if h1 != h0:
                        if h1 < nh:
                            a1 = head_window(h1)
                            d1 = vals[h1][0][lo - a1:hi - a1] * vals[h1][1]
                        else:
                            d1 = jnp.zeros((8, 128), F32)
                        d = jnp.where(row8 + lo < DH * h1, d, d1)
                    val = val + d
                rows.append(val)
            oT[g, :, qb * 128:(qb + 1) * 128] = jnp.concatenate(rows, axis=0).astype(BF16)

        order = (3, 2, 1, 0)
        for i, qb in enumerate(order):
            qk(qb, i % 2)
            if i > 0:
                pv(order[i - 1], (i - 1) % 2)
        pv(order[-1], (len(order) - 1) % 2)

    def _slow_attention():
        def g_body(g, c):
            oslow[...] = am[g]

            def j_body(j, c2):
                a = pl.multiple_of((DH * j // 16) * 16, 16)
                lo = DH * j

                def q_body(qb, c3):
                    q0 = pl.multiple_of(qb * 128, 128)
                    qt = qT_g[g, :, pl.ds(q0, 128)]
                    qm = jnp.where((r128 >= lo) & (r128 < lo + DH), qt, jnp.zeros_like(qt))
                    sc = jnp.dot(k_g[g], qm, preferred_element_type=F32)
                    ok = _iota((L, 128), 0) <= _iota((L, 128), 1) + q0
                    sc = jnp.where(ok, sc, -jnp.inf)
                    mx = jnp.max(sc, axis=0, keepdims=True)
                    p = jnp.exp2(sc - mx).astype(BF16)
                    vw = vT_g[g, pl.ds(a, 32), :]
                    vw = jnp.where(_iota((32, L), 0) == 31, jnp.ones_like(vw), vw)
                    acc = jnp.dot(vw, p, preferred_element_type=F32)
                    rr = _iota((32, 128), 0) + a
                    keep = (rr >= lo) & (rr < lo + DH)
                    gj = grep[g, pl.ds(a, 32), :]
                    val = acc * ((1.0 - gj) / acc[31:32])
                    cur = oslow[pl.ds(a, 32), pl.ds(q0, 128)]
                    oslow[pl.ds(a, 32), pl.ds(q0, 128)] = jnp.where(keep, cur + val, cur)
                    return c3
                return lax.fori_loop(0, 4, q_body, c2)
            lax.fori_loop(0, HPG, j_body, 0)
            oT[g] = oslow[...].astype(BF16)
            return c
        lax.fori_loop(0, NG, g_body, 0)

    lax.fori_loop(0, NSEG, seg_body, 0)

    rb = rb_ref[...]
    rmax = jnp.max(rb)
    idx = jnp.min(jnp.where(rb == rmax, ib_ref[...], SEQ))
    idx = jnp.clip(idx, 0, SEQ - 1)
    sg = idx // L
    t0 = pl.multiple_of(((idx % L) // 128) * 128, 128)
    hb = h_v[sg, :, pl.ds(t0, 128)]
    hf = hb.astype(F32)
    hn = _ln(hf).astype(BF16)
    hrow = jnp.concatenate([hn, jnp.zeros((DP - D, 128), BF16)], axis=0).T
    pick_r = _iota((128, DP), 0) == (idx % 128)
    xs = jnp.sum(jnp.where(pick_r, hrow.astype(F32), 0.0), axis=0, keepdims=True)
    xs = jnp.broadcast_to(xs[:, 0:D], (16, D)).astype(BF16)
    for i in range(3):
        f_copy(i).wait()
    gt = jnp.dot(xs, wg_v[...], preferred_element_type=F32)[0:8]
    up = jnp.dot(xs, wu_v[...], preferred_element_type=F32)[0:8]
    act = (gt * jax.nn.sigmoid(gt) * up)
    act = jnp.concatenate([act, act], axis=0).astype(BF16)
    y = lax.dot_general(act, wd_v[...], (((1,), (1,)), ((), ())),
                        preferred_element_type=F32)[0:1]
    y = y * jax.nn.sigmoid(jnp.full((1, D), rmax, F32))
    y = jnp.concatenate([y, jnp.zeros((1, DP - D), F32)], axis=1)
    ycol = jnp.broadcast_to(y, (128, DP)).T[0:D]
    hn = hn.astype(F32)
    new = (hf + (hn + ycol).astype(BF16).astype(F32)).astype(BF16)
    old = (hf + hn).astype(BF16)
    patch_v[...] = jnp.where(_iota((D, 128), 1) == (idx % 128), new, old)
    for s in range(NSEG):
        o_copy(s).wait()
    p0 = pl.multiple_of((idx // 128) * 128, 128)
    cp = pltpu.make_async_copy(patch_v, out_hbm.at[:, pl.ds(p0, 128)], sem_p)
    cp.start()
    cp.wait()


@jax.jit
def pallas_sequential_preLN__memory_aug_infini_attn__moe_arch_mod__prompt_kernel(
    A_x: jax.Array,
    A_wq: jax.Array,
    A_wk: jax.Array,
    A_wv: jax.Array,
    A_wo: jax.Array,
    A_beta: jax.Array,
    B_x: jax.Array,
    B_w_r: jax.Array,
    B_w_gate: jax.Array,
    B_w_up: jax.Array,
    B_w_down: jax.Array,
):
    del B_x
    hbm = pl.BlockSpec(memory_space=pltpu.HBM)
    VM = pltpu.VMEM
    outT = pl.pallas_call(
        _kernel,
        out_shape=jax.ShapeDtypeStruct((D, SEQ), BF16),
        in_specs=[hbm] * 10,
        out_specs=hbm,
        scratch_shapes=[
            VM((NSEG, D, L), BF16),
            VM((4, DP, D), BF16),
            VM((DP, DP), BF16),
            VM((3, QV_ROWS, DP), BF16),
            VM((D, DP), BF16),
            VM((D, FF), BF16),
            VM((D, FF), BF16),
            VM((D, FF), BF16),
            VM((H,), BF16),
            VM((D,), BF16),
            VM((DP, 128), F32),
            VM((NG, L, 128), BF16),
            VM((NG, 128, L), BF16),
            VM((NG, 128, L), BF16),
            VM((NG, 128, L), BF16),
            VM((NG, 128, L), BF16),
            VM((2, L, HPG * 128), BF16),
            VM((NG, 128, L), BF16),
            VM((NG, 128, L), F32),
            VM((NG, MROWS, 128), F32),
            VM((NG, 128, 128), F32),
            VM((NG, 8, 128), F32),
            VM((NSEG, D, L), BF16),
            VM((NSEG, D, L), BF16),
            VM((D, 128), BF16),
            VM((128, L), F32),
            VM((8, L), F32),
            VM((8, L), I32),
            pltpu.SemaphoreType.DMA((NSEG,)),
            pltpu.SemaphoreType.DMA((4,)),
            pltpu.SemaphoreType.DMA((3,)),
            pltpu.SemaphoreType.DMA((NSEG,)),
            pltpu.SemaphoreType.DMA(()),
            pltpu.SemaphoreType.DMA((2,)),
        ],
        compiler_params=pltpu.CompilerParams(vmem_limit_bytes=64 * 1024 * 1024),
    )(A_x.reshape(SEQ, D).T, A_wq, A_wk, A_wv, A_wo, A_beta, B_w_r,
      B_w_gate, B_w_up, B_w_down.T)
    return outT.T.reshape(1, SEQ, D)
```

```python
import functools

import jax
import jax.numpy as jnp
import numpy as np
from jax import lax
import jax.experimental.pallas as pl
import jax.experimental.pallas.tpu as pltpu

F32 = jnp.float32
BF16 = jnp.bfloat16
I32 = jnp.int32

SEQ = 2048
D = 576
DP = 640
H = 32
DH = 18
NSEG = 4
L = 512
FF = 4608
NG = 5
HPG = 7
LAST_ROWS = 80
QV_ROWS = 4 * 128 + LAST_ROWS
EPS = 1e-05
LOG2E = 1.4426950408889634
QSCALE = float(DH ** -0.5) * LOG2E
SAFE_BOUND = 40.0
V_BOUND = 2.0 ** 40
HD = D // 2
MROWS = 144


def _heads_in(g):
    return min(HPG, H - HPG * g)


def _iota(shape, dim):
    return lax.broadcasted_iota(I32, shape, dim)


def _pk(v):
    return pltpu.bitcast(v, I32)


def _up(w):
    return pltpu.bitcast(w, BF16)


def _blk(i, n):
    if isinstance(i, int):
        return slice(i * n, (i + 1) * n)
    return pl.ds(pl.multiple_of(i * n, 8), n)


def _unfold(ref, i, n):
    return jnp.concatenate([ref[_blk(i, n), 0:128], ref[_blk(i, n), 128:256]], axis=0)


def _f32(w):
    return _up(w).astype(F32)


def _ln_stats(w):
    lo = pltpu.bitcast(w << 16, F32)
    hi = pltpu.bitcast(w & jnp.int32(-65536), F32)
    piv = lo[0:1]
    dl = lo - piv
    dh = hi - piv
    n = 1.0 / (2 * w.shape[0])
    s1 = (jnp.sum(dl, axis=0, keepdims=True) + jnp.sum(dh, axis=0, keepdims=True)) * n
    s2 = (jnp.sum(dl * dl, axis=0, keepdims=True) + jnp.sum(dh * dh, axis=0, keepdims=True)) * n
    var = jnp.maximum(s2 - s1 * s1, 0.0)
    return piv + s1, lax.rsqrt(var + EPS)


def _phi(t):
    return jnp.where(t > 0, t + 1.0, jnp.exp(t))


def _kernel(x_hbm, wq_hbm, wk_hbm, wv_hbm, wo_hbm, beta_hbm, wr_hbm,
            wg_hbm, wu_hbm, wd_hbm, out_hbm,
            x_v, wraw, wtmp, wT, woT, wg_v, wu_v, wd_v, beta_v, wr_v, wr_col,
            k_g, pkT_g, qT_g, pqT_g, vT_g, p_buf, oT, am, MT, grep, omg,
            h_v, h2_v, patch_v, oslow, rb_ref, ib_ref, xn_v, ib_s,
            sem_x, sem_w, sem_f, sem_o, sem_p, sem_s):
    def x_copy(s):
        return pltpu.make_async_copy(x_hbm.at[:, pl.ds(s * L, L)], x_v.at[s], sem_x.at[s])

    def w_copy(i):
        src = (wq_hbm, wk_hbm, wv_hbm, wo_hbm)[i]
        return pltpu.make_async_copy(src, wraw.at[i, pl.ds(0, D), :], sem_w.at[i])

    def s_copy(i):
        src, dst = ((beta_hbm, beta_v), (wr_hbm, wr_v))[i]
        return pltpu.make_async_copy(src, dst, sem_s.at[i])

    def f_copy(i):
        src, dst = ((wg_hbm, wg_v), (wu_hbm, wu_v), (wd_hbm, wd_v))[i]
        return pltpu.make_async_copy(src, dst, sem_f.at[i])

    def o_copy(s):
        return pltpu.make_async_copy(h2_v.at[s], out_hbm.at[:, pl.ds(s * L, L)], sem_o.at[s])

    wraw[:, pl.ds(D, DP - D), :] = jnp.zeros((4, DP - D, D), BF16)
    w_copy(0).start()
    x_copy(0).start()
    w_copy(1).start()
    w_copy(2).start()
    s_copy(0).start()
    s_copy(1).start()
    w_copy(3).start()

    zi = jnp.zeros((64 - LAST_ROWS // 2, L), I32)
    for ref in (qT_g, pqT_g, pkT_g, vT_g):
        ref[QV_ROWS // 2:, :] = zi
    k_g[:, QV_ROWS:] = jnp.zeros((L // 2, DP - QV_ROWS), I32)
    ib_s[0] = 0
    rb_ref[...] = jnp.full((8, L), -jnp.inf, F32)
    ib_ref[...] = jnp.zeros((8, L), I32)

    def windows(src, dst, rows):
        keep = _iota((rows // 2, 128), 1) < HPG * DH
        for g in range(NG - 1):
            w = _pk(src[0:rows, HPG * DH * g: HPG * DH * g + 128])
            dst[0:rows // 2, 128 * g: 128 * (g + 1)] = jnp.where(keep, w, 0)
        dst[0:rows // 2, 512:640] = jnp.zeros((rows // 2, 128), I32)
        dst[0:rows // 2, 512:512 + 72] = _pk(src[0:rows, 504:576])

    for i in range(3):
        w_copy(i).wait()
        windows(wraw.at[i], wtmp, DP)
        wt = _up(wtmp[...]).T
        wT[_blk(i, QV_ROWS // 2), :] = _pk(wt[0:QV_ROWS, :])
    w_copy(3).wait()
    wtmp[:, 0:D] = _pk(wraw[3])
    wtmp[:, D:DP] = jnp.zeros((DP // 2, DP - D), I32)
    wraw[0, :, :] = _up(wtmp[...]).T[:, 0:D]
    windows(wraw.at[0], woT, D)

    for s in range(1, NSEG):
        x_copy(s).start()
    for i in range(3):
        f_copy(i).start()

    s_copy(0).wait()
    s_copy(1).wait()
    beta = beta_v[...].reshape(1, H).astype(F32)
    gate = jax.nn.sigmoid(beta)
    gate = jnp.concatenate([gate, jnp.zeros((1, 128 - H), F32)], axis=1)
    lane = _iota((128, 128), 1)
    row = _iota((128, 128), 0)
    lane8 = _iota((8, 128), 1)
    row8 = _iota((8, 128), 0)
    for g in range(NG):
        hid = HPG * g + row // DH
        sel = (lane == hid) & (row < _heads_in(g) * DH)
        gcol = jnp.sum(jnp.where(sel, jnp.broadcast_to(gate, (128, 128)), 0.0), axis=1, keepdims=True)
        grep[g] = jnp.broadcast_to(gcol, (128, 128))
        sel8 = (lane8 == HPG * g + row8) & (row8 < _heads_in(g))
        g8 = jnp.sum(jnp.where(sel8, jnp.broadcast_to(gate, (8, 128)), 0.0), axis=1, keepdims=True)
        omg[g] = jnp.broadcast_to(1.0 - g8, (8, 128))
    wr = wr_v[...].reshape(1, D).astype(F32)
    wr = jnp.concatenate([wr, jnp.zeros((1, DP - D), F32)], axis=1)
    wr_col[...] = jnp.broadcast_to(wr, (128, DP)).T

    r128 = _iota((128, 128), 0)
    c128 = _iota((128, 128), 1)
    mrow = _iota((MROWS, 128), 0)
    mlane = _iota((MROWS, 128), 1)
    mhead = jnp.where(mrow < 128, mrow // DH, mrow - 128)
    mmask = (mhead == mlane // DH) & (mlane < HPG * DH) & ((mrow < HPG * DH) | (mrow >= 128))
    ones16 = jnp.ones((16, L), BF16)
    kp = 2 * _iota((64, 128), 0)
    qc = _iota((64, 128), 1)
    causal = (jnp.where(kp <= qc, 0x0000FFFF, 0) | jnp.where(kp + 1 <= qc, jnp.int32(-65536), 0))

    def head_window(j):
        return (DH * j // 16) * 16

    def proj(i):
        xn = jnp.concatenate([_unfold(xn_v, c, D // 4) for c in range(L // 128)], axis=1)
        return lax.dot_general(_up(wT[_blk(i, QV_ROWS // 2), 0:D]), _up(xn), (((1,), (0,)), ((), ())),
                               preferred_element_type=F32)

    def ln_in(s):
        for c in range(L // 128):
            cs = slice(128 * c, 128 * (c + 1))
            m, rs = _ln_stats(_pk(x_v[s, :, cs]))
            xn_v[_blk(c, D // 4), :] = _pk(jnp.concatenate(
                [(x_v[s, 0:D // 2, cs].astype(F32) - m) * rs,
                 (x_v[s, D // 2:D, cs].astype(F32) - m) * rs], axis=1).astype(BF16))

    def out_proj_post(s):
        for c in range(L // 128):
            cs = slice(128 * c, 128 * (c + 1))
            ot = _up(jnp.concatenate([_unfold(oT, 4 * g + c, 32) for g in range(NG)], axis=0))
            hf = jnp.concatenate(
                [x_v[s, HD * u:HD * (u + 1), cs].astype(F32)
                 + jnp.dot(_up(woT[HD // 2 * u:HD // 2 * (u + 1), :]), ot, preferred_element_type=F32)
                 for u in range(2)], axis=1)
            h_v[_blk(4 * s + c, D // 4), :] = _pk(hf.astype(BF16))
            hw = _unfold(h_v, 4 * s + c + zero, D // 4)
            m, rs = _ln_stats(hw)
            hf = _f32(hw)
            hn = (hf - m) * rs
            h2_v[s, :, cs] = (hf + hn).astype(BF16)
            r = jnp.broadcast_to(jnp.sum(hn * wr_col[0:D, :], axis=0, keepdims=True), (8, 128))
            best = rb_ref[:, cs]
            upd = r > best
            rb_ref[:, cs] = jnp.where(upd, r, best)
            ib_ref[:, cs] = jnp.where(upd, lane8 + (s * L + 128 * c), ib_ref[:, cs])

    def seg_body(s):
        q = proj(0)
        qmax = jnp.max(jnp.abs(q))
        qT_g[0:QV_ROWS // 2, :] = _pk((q * QSCALE).astype(BF16))
        if s > 0:
            pqT_g[0:QV_ROWS // 2, :] = _pk(_phi(q).astype(BF16))
        k = proj(1)
        kmax = jnp.max(jnp.abs(k))
        k_g[:, 0:QV_ROWS] = _pk(k.astype(BF16).T)
        if s < NSEG - 1:
            pkT_g[0:QV_ROWS // 2, :] = _pk(_phi(k).astype(BF16))
        v = proj(2)
        vmax = jnp.max(jnp.abs(v))
        vT_g[0:QV_ROWS // 2, :] = _pk(v.astype(BF16))
        safe = (qmax * kmax * (DH * QSCALE * 1.02) <= SAFE_BOUND) & (vmax <= V_BOUND)

        for g in range(NG):
            _group(g, s)

        @pl.when(jnp.logical_not(safe))
        def _():
            _slow_attention()

        if s > 0:
            o_copy(s - 1).start()
        if s + 1 < NSEG:
            x_copy(s + 1).wait()
            ln_in(s + 1)
        out_proj_post(s)

    def _group(g, s):
        nh = _heads_in(g)
        g2 = slice(64 * g, 64 * (g + 1))
        mt = MT[g] if s > 0 else None
        if s > 0:
            gx = jnp.concatenate([grep[g], jnp.ones((MROWS - 128, 128), F32)], axis=0)
            mtb = jnp.where(mmask, mt * gx, 0.0).astype(BF16)
            nd = jnp.dot(mtb, _up(pqT_g[g2, :]), preferred_element_type=F32)
            rden = 1.0 / (nd[128:136] + 1e-06)
            for r in range(16):
                lo, hi = 8 * r, 8 * r + 8
                h0, h1 = lo // DH, min((hi - 1) // DH, HPG - 1)
                rd = jnp.broadcast_to(rden[h0:h0 + 1], (8, L))
                if h1 != h0:
                    rd = jnp.where(_iota((8, L), 0) + lo < DH * h1, rd,
                                   jnp.broadcast_to(rden[h1:h1 + 1], (8, L)))
                am[g, lo:hi, :] = nd[lo:hi] * rd
        else:
            am[g] = jnp.zeros((128, L), F32)
        if s < NSEG - 1:
            lhs = jnp.concatenate([_up(vT_g[g2, :]), ones16], axis=0)
            upd = lax.dot_general(lhs, _up(pkT_g[g2, :]), (((1,), (1,)), ((), ())),
                                  preferred_element_type=F32)
            MT[g] = upd if s == 0 else mt + upd

        def qk(qb, slot):
            nk = (qb + 1) * 128
            qt = qT_g[g2, qb * 128:(qb + 1) * 128]
            rr = _iota((64, 128), 0)
            qm = _up(jnp.concatenate(
                [jnp.where((rr >= 9 * j) & (rr < 9 * j + 9), qt, 0)
                 for j in range(nh)], axis=1))
            sc = jnp.dot(_up(k_g[0:nk // 2, 128 * g:128 * (g + 1)]), qm, preferred_element_type=F32)
            p_buf[256 * slot:256 * slot + nk // 2, 0:nh * 128] = _pk(jnp.exp2(sc).astype(BF16))

        def pv(qb, slot):
            nk = (qb + 1) * 128
            vals = []
            for j in range(nh):
                a2 = 64 * g + head_window(j) // 2
                vw = vT_g[a2:a2 + 16, 0:nk]
                vw = jnp.where(_iota((16, nk), 0) == 15, 0x3F803F80, vw)
                js = slice(j * 128, (j + 1) * 128)
                p0 = 256 * slot
                pw = p_buf[p0 + (nk - 128) // 2:p0 + nk // 2, js] & causal
                if nk > 128:
                    pw = jnp.concatenate([p_buf[p0:p0 + (nk - 128) // 2, js], pw], axis=0)
                acc = jnp.dot(_up(vw), _up(pw), preferred_element_type=F32)
                rd = omg[g, j:j + 1, :] / acc[31:32]
                vals.append((acc, jnp.broadcast_to(rd, (8, 128))))
            rows = []
            for r in range(16):
                lo, hi = 8 * r, 8 * r + 8
                h0, h1 = lo // DH, (hi - 1) // DH
                val = am[g, lo:hi, qb * 128:(qb + 1) * 128] if s > 0 else None
                if h0 < nh:
                    a0 = head_window(h0)
                    d = vals[h0][0][lo - a0:hi - a0] * vals[h0][1]
                    if h1 != h0:
                        if h1 < nh:
                            a1 = head_window(h1)
                            d1 = vals[h1][0][lo - a1:hi - a1] * vals[h1][1]
                        else:
                            d1 = jnp.zeros((8, 128), F32)
                        d = jnp.where(row8 + lo < DH * h1, d, d1)
                    val = d if val is None else val + d
                elif val is None:
                    val = jnp.zeros((8, 128), F32)
                rows.append(val)
            oT[_blk(4 * g + qb, 32), :] = _pk(jnp.concatenate(
                [jnp.concatenate(rows[:8], axis=0), jnp.concatenate(rows[8:], axis=0)],
                axis=1).astype(BF16))

        order = (3, 2, 1, 0)
        for i, qb in enumerate(order):
            qk(qb, i % 2)
            if i > 0:
                pv(order[i - 1], (i - 1) % 2)
        pv(order[-1], (len(order) - 1) % 2)

    def _slow_attention():
        def g_body(g, c):
            oslow[...] = am[g]

            def j_body(j, c2):
                a = pl.multiple_of((DH * j // 16) * 16, 16)
                a2 = pl.multiple_of((DH * j // 16) * 8, 8)
                lo = DH * j

                def q_body(qb, c3):
                    q0 = pl.multiple_of(qb * 128, 128)
                    g64 = pl.multiple_of(g * 64, 64)
                    qt = _up(qT_g[pl.ds(g64, 64), pl.ds(q0, 128)])
                    qm = jnp.where((r128 >= lo) & (r128 < lo + DH), qt, jnp.zeros_like(qt))
                    sc = jnp.dot(_up(k_g[:, pl.ds(pl.multiple_of(g * 128, 128), 128)]), qm,
                                 preferred_element_type=F32)
                    ok = _iota((L, 128), 0) <= _iota((L, 128), 1) + q0
                    sc = jnp.where(ok, sc, -jnp.inf)
                    mx = jnp.max(sc, axis=0, keepdims=True)
                    p = jnp.exp2(sc - mx).astype(BF16)
                    vw = _up(vT_g[pl.ds(pl.multiple_of(g64 + a2, 8), 16), :])
                    vw = jnp.where(_iota((32, L), 0) == 31, jnp.ones_like(vw), vw)
                    acc = jnp.dot(vw, p, preferred_element_type=F32)
                    rr = _iota((32, 128), 0) + a
                    keep = (rr >= lo) & (rr < lo + DH)
                    gj = grep[g, pl.ds(a, 32), :]
                    val = acc * ((1.0 - gj) / acc[31:32])
                    cur = oslow[pl.ds(a, 32), pl.ds(q0, 128)]
                    oslow[pl.ds(a, 32), pl.ds(q0, 128)] = jnp.where(keep, cur + val, cur)
                    return c3
                return lax.fori_loop(0, 4, q_body, c2)
            lax.fori_loop(0, HPG, j_body, 0)
            for qb in range(4):
                qs = slice(128 * qb, 128 * (qb + 1))
                oT[_blk(4 * g + qb, 32), :] = _pk(
                    jnp.concatenate([oslow[0:64, qs], oslow[64:128, qs]], axis=1).astype(BF16))
            return c
        lax.fori_loop(0, NG, g_body, 0)

    zero = ib_s[0]
    x_copy(0).wait()
    ln_in(0)
    for s in range(NSEG):
        seg_body(s)

    o_copy(NSEG - 1).start()
    rb = rb_ref[...]
    rmax = jnp.max(rb)
    idx = jnp.min(jnp.where(rb == rmax, ib_ref[...], SEQ))
    idx = jnp.clip(idx, 0, SEQ - 1)
    hw = _unfold(h_v, idx // 128, D // 4)
    m, rs = _ln_stats(hw)
    hf = _up(hw).astype(F32)
    hn = ((hf - m) * rs).astype(BF16)
    hrow = jnp.concatenate([hn, jnp.zeros((DP - D, 128), BF16)], axis=0).T
    pick_r = _iota((128, DP), 0) == (idx % 128)
    xs = jnp.sum(jnp.where(pick_r, hrow.astype(F32), 0.0), axis=0, keepdims=True)
    xs = jnp.broadcast_to(xs[:, 0:D], (16, D)).astype(BF16)
    for i in range(3):
        f_copy(i).wait()
    gt = jnp.dot(xs, wg_v[...], preferred_element_type=F32)[0:8]
    up = jnp.dot(xs, wu_v[...], preferred_element_type=F32)[0:8]
    act = (gt * jax.nn.sigmoid(gt) * up)
    act = jnp.concatenate([act, act], axis=0).astype(BF16)
    y = lax.dot_general(act, wd_v[...], (((1,), (1,)), ((), ())),
                        preferred_element_type=F32)[0:1]
    y = y * jax.nn.sigmoid(jnp.full((1, D), rmax, F32))
    y = jnp.concatenate([y, jnp.zeros((1, DP - D), F32)], axis=1)
    ycol = jnp.broadcast_to(y, (128, DP)).T[0:D]
    hn = hn.astype(F32)
    new = (hf + (hn + ycol).astype(BF16).astype(F32)).astype(BF16)
    old = (hf + hn).astype(BF16)
    patch_v[...] = jnp.where(_iota((D, 128), 1) == (idx % 128), new, old)
    for s in range(NSEG):
        o_copy(s).wait()
    p0 = pl.multiple_of((idx // 128) * 128, 128)
    cp = pltpu.make_async_copy(patch_v, out_hbm.at[:, pl.ds(p0, 128)], sem_p)
    cp.start()
    cp.wait()


@jax.jit
def pallas_sequential_preLN__memory_aug_infini_attn__moe_arch_mod__prompt_kernel(
    A_x: jax.Array,
    A_wq: jax.Array,
    A_wk: jax.Array,
    A_wv: jax.Array,
    A_wo: jax.Array,
    A_beta: jax.Array,
    B_x: jax.Array,
    B_w_r: jax.Array,
    B_w_gate: jax.Array,
    B_w_up: jax.Array,
    B_w_down: jax.Array,
):
    del B_x
    hbm = pl.BlockSpec(memory_space=pltpu.HBM)
    VM = pltpu.VMEM
    outT = pl.pallas_call(
        _kernel,
        out_shape=jax.ShapeDtypeStruct((D, SEQ), BF16),
        in_specs=[hbm] * 10,
        out_specs=hbm,
        scratch_shapes=[
            VM((NSEG, D, L), BF16),
            VM((4, DP, D), BF16),
            VM((DP // 2, DP), I32),
            VM((3 * QV_ROWS // 2, DP), I32),
            VM((D // 2, DP), I32),
            VM((D, FF), BF16),
            VM((D, FF), BF16),
            VM((D, FF), BF16),
            VM((H,), BF16),
            VM((D,), BF16),
            VM((DP, 128), F32),
            VM((L // 2, DP), I32),
            VM((NG * 64, L), I32),
            VM((NG * 64, L), I32),
            VM((NG * 64, L), I32),
            VM((NG * 64, L), I32),
            VM((L, HPG * 128), I32),
            VM((NG * 4 * 32, 256), I32),
            VM((NG, 128, L), F32),
            VM((NG, MROWS, 128), F32),
            VM((NG, 128, 128), F32),
            VM((NG, 8, 128), F32),
            VM((NSEG * D, 256), I32),
            VM((NSEG, D, L), BF16),
            VM((D, 128), BF16),
            VM((128, L), F32),
            VM((8, L), F32),
            VM((8, L), I32),
            VM((D, 256), I32),
            pltpu.SMEM((1,), I32),
            pltpu.SemaphoreType.DMA((NSEG,)),
            pltpu.SemaphoreType.DMA((4,)),
            pltpu.SemaphoreType.DMA((3,)),
            pltpu.SemaphoreType.DMA((NSEG,)),
            pltpu.SemaphoreType.DMA(()),
            pltpu.SemaphoreType.DMA((2,)),
        ],
        compiler_params=pltpu.CompilerParams(vmem_limit_bytes=64 * 1024 * 1024),
    )(A_x.reshape(SEQ, D).T, A_wq, A_wk, A_wv, A_wo, A_beta, B_w_r,
      B_w_gate, B_w_up, B_w_down.T)
    return outT.T.reshape(1, SEQ, D)
```

```python
import functools

import jax
import jax.numpy as jnp
import numpy as np
from jax import lax
import jax.experimental.pallas as pl
import jax.experimental.pallas.tpu as pltpu

F32 = jnp.float32
BF16 = jnp.bfloat16
I32 = jnp.int32

SEQ = 2048
D = 576
DP = 640
H = 32
DH = 18
NSEG = 4
L = 512
FF = 4608
NG = 5
HPG = 7
LAST_ROWS = 80
QV_ROWS = 4 * 128 + LAST_ROWS
EPS = 1e-05
LOG2E = 1.4426950408889634
QSCALE = float(DH ** -0.5) * LOG2E
SAFE_BOUND = 40.0
V_BOUND = 2.0 ** 40
HD = D // 2
MROWS = 144


def _heads_in(g):
    return min(HPG, H - HPG * g)


def _iota(shape, dim):
    return lax.broadcasted_iota(I32, shape, dim)


def _pk(v):
    return pltpu.bitcast(v, I32)


def _up(w):
    return pltpu.bitcast(w, BF16)


def _blk(i, n):
    if isinstance(i, int):
        return slice(i * n, (i + 1) * n)
    return pl.ds(pl.multiple_of(i * n, 8), n)


def _unfold(ref, i, n):
    return jnp.concatenate([ref[_blk(i, n), 0:128], ref[_blk(i, n), 128:256]], axis=0)


def _f32(w):
    return _up(w).astype(F32)


def _ln_stats(w):
    lo = pltpu.bitcast(w << 16, F32)
    hi = pltpu.bitcast(w & jnp.int32(-65536), F32)
    piv = lo[0:1]
    dl = lo - piv
    dh = hi - piv
    n = 1.0 / (2 * w.shape[0])
    s1 = (jnp.sum(dl, axis=0, keepdims=True) + jnp.sum(dh, axis=0, keepdims=True)) * n
    s2 = (jnp.sum(dl * dl, axis=0, keepdims=True) + jnp.sum(dh * dh, axis=0, keepdims=True)) * n
    var = jnp.maximum(s2 - s1 * s1, 0.0)
    return piv + s1, lax.rsqrt(var + EPS)


def _phi(t):
    return jnp.where(t > 0, t + 1.0, jnp.exp(t))


def _kernel(x_hbm, wq_hbm, wk_hbm, wv_hbm, wo_hbm, beta_hbm, wr_hbm,
            wg_hbm, wu_hbm, wd_hbm, out_hbm,
            x_v, wraw, wtmp, wT, woT, wg_v, wu_v, wd_v, beta_v, wr_v, wr_col,
            k_g, pkT_g, qT_g, pqT_g, vT_g, p_buf, oT, am, MT, grep, omg,
            h_v, h2_v, patch_v, oslow, rb_ref, ib_ref, xn_v, ib_s,
            sem_x, sem_w, sem_f, sem_o, sem_p, sem_s):
    def x_copy(s):
        return pltpu.make_async_copy(x_hbm.at[:, pl.ds(pl.multiple_of(s * L, L), L)], x_v.at[s], sem_x.at[s])

    def w_copy(i):
        src = (wq_hbm, wk_hbm, wv_hbm, wo_hbm)[i]
        return pltpu.make_async_copy(src, wraw.at[i, pl.ds(0, D), :], sem_w.at[i])

    def s_copy(i):
        src, dst = ((beta_hbm, beta_v), (wr_hbm, wr_v))[i]
        return pltpu.make_async_copy(src, dst, sem_s.at[i])

    def f_copy(i):
        src, dst = ((wg_hbm, wg_v), (wu_hbm, wu_v), (wd_hbm, wd_v))[i]
        return pltpu.make_async_copy(src, dst, sem_f.at[i])

    def o_copy(s):
        return pltpu.make_async_copy(h2_v.at[s], out_hbm.at[:, pl.ds(pl.multiple_of(s * L, L), L)], sem_o.at[s])

    wraw[:, pl.ds(D, DP - D), :] = jnp.zeros((4, DP - D, D), BF16)
    w_copy(0).start()
    x_copy(0).start()
    w_copy(1).start()
    w_copy(2).start()
    s_copy(0).start()
    s_copy(1).start()
    w_copy(3).start()

    zi = jnp.zeros((64 - LAST_ROWS // 2, L), I32)
    for ref in (qT_g, pqT_g, pkT_g, vT_g):
        ref[QV_ROWS // 2:, :] = zi
    k_g[:, QV_ROWS:] = jnp.zeros((L // 2, DP - QV_ROWS), I32)
    ib_s[0] = 0
    MT[...] = jnp.zeros(MT.shape, F32)
    rb_ref[...] = jnp.full((8, L), -jnp.inf, F32)
    ib_ref[...] = jnp.zeros((8, L), I32)

    def windows(src, dst, rows):
        keep = _iota((rows // 2, 128), 1) < HPG * DH
        for g in range(NG - 1):
            w = _pk(src[0:rows, HPG * DH * g: HPG * DH * g + 128])
            dst[0:rows // 2, 128 * g: 128 * (g + 1)] = jnp.where(keep, w, 0)
        dst[0:rows // 2, 512:640] = jnp.zeros((rows // 2, 128), I32)
        dst[0:rows // 2, 512:512 + 72] = _pk(src[0:rows, 504:576])

    for i in range(3):
        w_copy(i).wait()
        windows(wraw.at[i], wtmp, DP)
        wt = _up(wtmp[...]).T
        wT[_blk(i, QV_ROWS // 2), :] = _pk(wt[0:QV_ROWS, :])
    w_copy(3).wait()
    wtmp[:, 0:D] = _pk(wraw[3])
    wtmp[:, D:DP] = jnp.zeros((DP // 2, DP - D), I32)
    wraw[0, :, :] = _up(wtmp[...]).T[:, 0:D]
    windows(wraw.at[0], woT, D)

    for s in range(1, NSEG):
        x_copy(s).start()
    for i in range(3):
        f_copy(i).start()

    s_copy(0).wait()
    s_copy(1).wait()
    beta = beta_v[...].reshape(1, H).astype(F32)
    gate = jax.nn.sigmoid(beta)
    gate = jnp.concatenate([gate, jnp.zeros((1, 128 - H), F32)], axis=1)
    lane = _iota((128, 128), 1)
    row = _iota((128, 128), 0)
    lane8 = _iota((8, 128), 1)
    row8 = _iota((8, 128), 0)
    for g in range(NG):
        hid = HPG * g + row // DH
        sel = (lane == hid) & (row < _heads_in(g) * DH)
        gcol = jnp.sum(jnp.where(sel, jnp.broadcast_to(gate, (128, 128)), 0.0), axis=1, keepdims=True)
        grep[g] = jnp.broadcast_to(gcol, (128, 128))
        sel8 = (lane8 == HPG * g + row8) & (row8 < _heads_in(g))
        g8 = jnp.sum(jnp.where(sel8, jnp.broadcast_to(gate, (8, 128)), 0.0), axis=1, keepdims=True)
        omg[g] = jnp.broadcast_to(1.0 - g8, (8, 128))
    wr = wr_v[...].reshape(1, D).astype(F32)
    wr = jnp.concatenate([wr, jnp.zeros((1, DP - D), F32)], axis=1)
    wr_col[...] = jnp.broadcast_to(wr, (128, DP)).T

    r128 = _iota((128, 128), 0)
    c128 = _iota((128, 128), 1)
    mrow = _iota((MROWS, 128), 0)
    mlane = _iota((MROWS, 128), 1)
    mhead = jnp.where(mrow < 128, mrow // DH, mrow - 128)
    mmask = (mhead == mlane // DH) & (mlane < HPG * DH) & ((mrow < HPG * DH) | (mrow >= 128))
    ones16 = jnp.ones((16, L), BF16)
    kp = 2 * _iota((64, 128), 0)
    qc = _iota((64, 128), 1)
    causal = (jnp.where(kp <= qc, 0x0000FFFF, 0) | jnp.where(kp + 1 <= qc, jnp.int32(-65536), 0))

    def head_window(j):
        return (DH * j // 16) * 16

    def proj(i):
        xn = jnp.concatenate([_unfold(xn_v, c, D // 4) for c in range(L // 128)], axis=1)
        return lax.dot_general(_up(wT[_blk(i, QV_ROWS // 2), 0:D]), _up(xn), (((1,), (0,)), ((), ())),
                               preferred_element_type=F32)

    def ln_in(s):
        for c in range(L // 128):
            cs = slice(128 * c, 128 * (c + 1))
            m, rs = _ln_stats(_pk(x_v[s, :, cs]))
            xn_v[_blk(c, D // 4), :] = _pk(jnp.concatenate(
                [(x_v[s, 0:D // 2, cs].astype(F32) - m) * rs,
                 (x_v[s, D // 2:D, cs].astype(F32) - m) * rs], axis=1).astype(BF16))

    def out_proj_post(s):
        for c in range(L // 128):
            cs = slice(128 * c, 128 * (c + 1))
            ot = _up(jnp.concatenate([_unfold(oT, 4 * g + c, 32) for g in range(NG)], axis=0))
            hf = jnp.concatenate(
                [x_v[s, HD * u:HD * (u + 1), cs].astype(F32)
                 + jnp.dot(_up(woT[HD // 2 * u:HD // 2 * (u + 1), :]), ot, preferred_element_type=F32)
                 for u in range(2)], axis=1)
            h_v[_blk(4 * s + c, D // 4), :] = _pk(hf.astype(BF16))
            hw = _unfold(h_v, 4 * s + c + zero, D // 4)
            m, rs = _ln_stats(hw)
            hf = _f32(hw)
            hn = (hf - m) * rs
            h2_v[s, :, cs] = (hf + hn).astype(BF16)
            r = jnp.broadcast_to(jnp.sum(hn * wr_col[0:D, :], axis=0, keepdims=True), (8, 128))
            best = rb_ref[:, cs]
            upd = r > best
            rb_ref[:, cs] = jnp.where(upd, r, best)
            ib_ref[:, cs] = jnp.where(upd, lane8 + (s * L + 128 * c), ib_ref[:, cs])

    def seg_body(s):
        q = proj(0)
        qmax = jnp.max(jnp.abs(q))
        qT_g[0:QV_ROWS // 2, :] = _pk((q * QSCALE).astype(BF16))
        if True:
            pqT_g[0:QV_ROWS // 2, :] = _pk(_phi(q).astype(BF16))
        k = proj(1)
        kmax = jnp.max(jnp.abs(k))
        k_g[:, 0:QV_ROWS] = _pk(k.astype(BF16).T)
        if True:
            pkT_g[0:QV_ROWS // 2, :] = _pk(_phi(k).astype(BF16))
        v = proj(2)
        vmax = jnp.max(jnp.abs(v))
        vT_g[0:QV_ROWS // 2, :] = _pk(v.astype(BF16))
        safe = (qmax * kmax * (DH * QSCALE * 1.02) <= SAFE_BOUND) & (vmax <= V_BOUND)

        for g in range(NG):
            _group(g, 1)

        @pl.when(jnp.logical_not(safe))
        def _():
            _slow_attention()

        @pl.when(s > 0)
        def _():
            o_copy(s - 1).start()

        @pl.when(s + 1 < NSEG)
        def _():
            x_copy(s + 1).wait()
        ln_in(jnp.minimum(s + 1, NSEG - 1))
        out_proj_post(s)

    def _group(g, s):
        nh = _heads_in(g)
        g2 = slice(64 * g, 64 * (g + 1))
        mt = MT[g] if s > 0 else None
        if s > 0:
            gx = jnp.concatenate([grep[g], jnp.ones((MROWS - 128, 128), F32)], axis=0)
            mtb = jnp.where(mmask, mt * gx, 0.0).astype(BF16)
            nd = jnp.dot(mtb, _up(pqT_g[g2, :]), preferred_element_type=F32)
            rden = 1.0 / (nd[128:136] + 1e-06)
            for r in range(16):
                lo, hi = 8 * r, 8 * r + 8
                h0, h1 = lo // DH, min((hi - 1) // DH, HPG - 1)
                rd = jnp.broadcast_to(rden[h0:h0 + 1], (8, L))
                if h1 != h0:
                    rd = jnp.where(_iota((8, L), 0) + lo < DH * h1, rd,
                                   jnp.broadcast_to(rden[h1:h1 + 1], (8, L)))
                am[g, lo:hi, :] = nd[lo:hi] * rd
        else:
            am[g] = jnp.zeros((128, L), F32)
        if s < NSEG - 1:
            lhs = jnp.concatenate([_up(vT_g[g2, :]), ones16], axis=0)
            upd = lax.dot_general(lhs, _up(pkT_g[g2, :]), (((1,), (1,)), ((), ())),
                                  preferred_element_type=F32)
            MT[g] = upd if s == 0 else mt + upd

        def qk(qb, slot):
            nk = (qb + 1) * 128
            qt = qT_g[g2, qb * 128:(qb + 1) * 128]
            rr = _iota((64, 128), 0)
            qm = _up(jnp.concatenate(
                [jnp.where((rr >= 9 * j) & (rr < 9 * j + 9), qt, 0)
                 for j in range(nh)], axis=1))
            sc = jnp.dot(_up(k_g[0:nk // 2, 128 * g:128 * (g + 1)]), qm, preferred_element_type=F32)
            p_buf[256 * slot:256 * slot + nk // 2, 0:nh * 128] = _pk(jnp.exp2(sc).astype(BF16))

        def pv(qb, slot):
            nk = (qb + 1) * 128
            vals = []
            for j in range(nh):
                a2 = 64 * g + head_window(j) // 2
                vw = vT_g[a2:a2 + 16, 0:nk]
                vw = jnp.where(_iota((16, nk), 0) == 15, 0x3F803F80, vw)
                js = slice(j * 128, (j + 1) * 128)
                p0 = 256 * slot
                pw = p_buf[p0 + (nk - 128) // 2:p0 + nk // 2, js] & causal
                if nk > 128:
                    pw = jnp.concatenate([p_buf[p0:p0 + (nk - 128) // 2, js], pw], axis=0)
                acc = jnp.dot(_up(vw), _up(pw), preferred_element_type=F32)
                rd = omg[g, j:j + 1, :] / acc[31:32]
                vals.append((acc, jnp.broadcast_to(rd, (8, 128))))
            rows = []
            for r in range(16):
                lo, hi = 8 * r, 8 * r + 8
                h0, h1 = lo // DH, (hi - 1) // DH
                val = am[g, lo:hi, qb * 128:(qb + 1) * 128] if s > 0 else None
                if h0 < nh:
                    a0 = head_window(h0)
                    d = vals[h0][0][lo - a0:hi - a0] * vals[h0][1]
                    if h1 != h0:
                        if h1 < nh:
                            a1 = head_window(h1)
                            d1 = vals[h1][0][lo - a1:hi - a1] * vals[h1][1]
                        else:
                            d1 = jnp.zeros((8, 128), F32)
                        d = jnp.where(row8 + lo < DH * h1, d, d1)
                    val = d if val is None else val + d
                elif val is None:
                    val = jnp.zeros((8, 128), F32)
                rows.append(val)
            oT[_blk(4 * g + qb, 32), :] = _pk(jnp.concatenate(
                [jnp.concatenate(rows[:8], axis=0), jnp.concatenate(rows[8:], axis=0)],
                axis=1).astype(BF16))

        order = (3, 2, 1, 0)
        for i, qb in enumerate(order):
            qk(qb, i % 2)
            if i > 0:
                pv(order[i - 1], (i - 1) % 2)
        pv(order[-1], (len(order) - 1) % 2)

    def _slow_attention():
        def g_body(g, c):
            oslow[...] = am[g]

            def j_body(j, c2):
                a = pl.multiple_of((DH * j // 16) * 16, 16)
                a2 = pl.multiple_of((DH * j // 16) * 8, 8)
                lo = DH * j

                def q_body(qb, c3):
                    q0 = pl.multiple_of(qb * 128, 128)
                    g64 = pl.multiple_of(g * 64, 64)
                    qt = _up(qT_g[pl.ds(g64, 64), pl.ds(q0, 128)])
                    qm = jnp.where((r128 >= lo) & (r128 < lo + DH), qt, jnp.zeros_like(qt))
                    sc = jnp.dot(_up(k_g[:, pl.ds(pl.multiple_of(g * 128, 128), 128)]), qm,
                                 preferred_element_type=F32)
                    ok = _iota((L, 128), 0) <= _iota((L, 128), 1) + q0
                    sc = jnp.where(ok, sc, -jnp.inf)
                    mx = jnp.max(sc, axis=0, keepdims=True)
                    p = jnp.exp2(sc - mx).astype(BF16)
                    vw = _up(vT_g[pl.ds(pl.multiple_of(g64 + a2, 8), 16), :])
                    vw = jnp.where(_iota((32, L), 0) == 31, jnp.ones_like(vw), vw)
                    acc = jnp.dot(vw, p, preferred_element_type=F32)
                    rr = _iota((32, 128), 0) + a
                    keep = (rr >= lo) & (rr < lo + DH)
                    gj = grep[g, pl.ds(a, 32), :]
                    val = acc * ((1.0 - gj) / acc[31:32])
                    cur = oslow[pl.ds(a, 32), pl.ds(q0, 128)]
                    oslow[pl.ds(a, 32), pl.ds(q0, 128)] = jnp.where(keep, cur + val, cur)
                    return c3
                return lax.fori_loop(0, 4, q_body, c2)
            lax.fori_loop(0, HPG, j_body, 0)
            for qb in range(4):
                qs = slice(128 * qb, 128 * (qb + 1))
                oT[_blk(4 * g + qb, 32), :] = _pk(
                    jnp.concatenate([oslow[0:64, qs], oslow[64:128, qs]], axis=1).astype(BF16))
            return c
        lax.fori_loop(0, NG, g_body, 0)

    zero = ib_s[0]
    x_copy(0).wait()
    ln_in(0)
    lax.fori_loop(0, NSEG, lambda s, c: (seg_body(s), c)[1], 0)

    o_copy(NSEG - 1).start()
    rb = rb_ref[...]
    rmax = jnp.max(rb)
    idx = jnp.min(jnp.where(rb == rmax, ib_ref[...], SEQ))
    idx = jnp.clip(idx, 0, SEQ - 1)
    hw = _unfold(h_v, idx // 128, D // 4)
    m, rs = _ln_stats(hw)
    hf = _up(hw).astype(F32)
    hn = ((hf - m) * rs).astype(BF16)
    hrow = jnp.concatenate([hn, jnp.zeros((DP - D, 128), BF16)], axis=0).T
    pick_r = _iota((128, DP), 0) == (idx % 128)
    xs = jnp.sum(jnp.where(pick_r, hrow.astype(F32), 0.0), axis=0, keepdims=True)
    xs = jnp.broadcast_to(xs[:, 0:D], (16, D)).astype(BF16)
    for i in range(3):
        f_copy(i).wait()
    gt = jnp.dot(xs, wg_v[...], preferred_element_type=F32)[0:8]
    up = jnp.dot(xs, wu_v[...], preferred_element_type=F32)[0:8]
    act = (gt * jax.nn.sigmoid(gt) * up)
    act = jnp.concatenate([act, act], axis=0).astype(BF16)
    y = lax.dot_general(act, wd_v[...], (((1,), (1,)), ((), ())),
                        preferred_element_type=F32)[0:1]
    y = y * jax.nn.sigmoid(jnp.full((1, D), rmax, F32))
    y = jnp.concatenate([y, jnp.zeros((1, DP - D), F32)], axis=1)
    ycol = jnp.broadcast_to(y, (128, DP)).T[0:D]
    hn = hn.astype(F32)
    new = (hf + (hn + ycol).astype(BF16).astype(F32)).astype(BF16)
    old = (hf + hn).astype(BF16)
    patch_v[...] = jnp.where(_iota((D, 128), 1) == (idx % 128), new, old)
    for s in range(NSEG):
        o_copy(s).wait()
    p0 = pl.multiple_of((idx // 128) * 128, 128)
    cp = pltpu.make_async_copy(patch_v, out_hbm.at[:, pl.ds(p0, 128)], sem_p)
    cp.start()
    cp.wait()


@jax.jit
def pallas_sequential_preLN__memory_aug_infini_attn__moe_arch_mod__prompt_kernel(
    A_x: jax.Array,
    A_wq: jax.Array,
    A_wk: jax.Array,
    A_wv: jax.Array,
    A_wo: jax.Array,
    A_beta: jax.Array,
    B_x: jax.Array,
    B_w_r: jax.Array,
    B_w_gate: jax.Array,
    B_w_up: jax.Array,
    B_w_down: jax.Array,
):
    del B_x
    hbm = pl.BlockSpec(memory_space=pltpu.HBM)
    VM = pltpu.VMEM
    outT = pl.pallas_call(
        _kernel,
        out_shape=jax.ShapeDtypeStruct((D, SEQ), BF16),
        in_specs=[hbm] * 10,
        out_specs=hbm,
        scratch_shapes=[
            VM((NSEG, D, L), BF16),
            VM((4, DP, D), BF16),
            VM((DP // 2, DP), I32),
            VM((3 * QV_ROWS // 2, DP), I32),
            VM((D // 2, DP), I32),
            VM((D, FF), BF16),
            VM((D, FF), BF16),
            VM((D, FF), BF16),
            VM((H,), BF16),
            VM((D,), BF16),
            VM((DP, 128), F32),
            VM((L // 2, DP), I32),
            VM((NG * 64, L), I32),
            VM((NG * 64, L), I32),
            VM((NG * 64, L), I32),
            VM((NG * 64, L), I32),
            VM((L, HPG * 128), I32),
            VM((NG * 4 * 32, 256), I32),
            VM((NG, 128, L), F32),
            VM((NG, MROWS, 128), F32),
            VM((NG, 128, 128), F32),
            VM((NG, 8, 128), F32),
            VM((NSEG * D, 256), I32),
            VM((NSEG, D, L), BF16),
            VM((D, 128), BF16),
            VM((128, L), F32),
            VM((8, L), F32),
            VM((8, L), I32),
            VM((D, 256), I32),
            pltpu.SMEM((1,), I32),
            pltpu.SemaphoreType.DMA((NSEG,)),
            pltpu.SemaphoreType.DMA((4,)),
            pltpu.SemaphoreType.DMA((3,)),
            pltpu.SemaphoreType.DMA((NSEG,)),
            pltpu.SemaphoreType.DMA(()),
            pltpu.SemaphoreType.DMA((2,)),
        ],
        compiler_params=pltpu.CompilerParams(vmem_limit_bytes=64 * 1024 * 1024),
    )(A_x.reshape(SEQ, D).T, A_wq, A_wk, A_wv, A_wo, A_beta, B_w_r,
      B_w_gate, B_w_up, B_w_down.T)
    return outT.T.reshape(1, SEQ, D)
```

```python
import functools

import jax
import jax.numpy as jnp
import numpy as np
from jax import lax
import jax.experimental.pallas as pl
import jax.experimental.pallas.tpu as pltpu

F32 = jnp.float32
BF16 = jnp.bfloat16
I32 = jnp.int32

SEQ = 2048
D = 576
DP = 640
H = 32
DH = 18
NSEG = 4
L = 512
FF = 4608
NG = 5
HPG = 7
LAST_ROWS = 80
QV_ROWS = 4 * 128 + LAST_ROWS
EPS = 1e-05
LOG2E = 1.4426950408889634
QSCALE = float(DH ** -0.5) * LOG2E
SAFE_BOUND = 40.0
V_BOUND = 2.0 ** 40
HD = D // 2
MROWS = 136


def _heads_in(g):
    return min(HPG, H - HPG * g)


def _iota(shape, dim):
    return lax.broadcasted_iota(I32, shape, dim)


def _pk(v):
    return pltpu.bitcast(v, I32)


def _up(w):
    return pltpu.bitcast(w, BF16)


def _blk(i, n):
    if isinstance(i, int):
        return slice(i * n, (i + 1) * n)
    return pl.ds(pl.multiple_of(i * n, 8), n)


def _unfold(ref, i, n):
    return jnp.concatenate([ref[_blk(i, n), 0:128], ref[_blk(i, n), 128:256]], axis=0)


def _f32(w):
    return _up(w).astype(F32)


def _ln_stats(w):
    lo = pltpu.bitcast(w << 16, F32)
    hi = pltpu.bitcast(w & jnp.int32(-65536), F32)
    piv = lo[0:1]
    dl = lo - piv
    dh = hi - piv
    n = 1.0 / (2 * w.shape[0])
    s1 = (jnp.sum(dl, axis=0, keepdims=True) + jnp.sum(dh, axis=0, keepdims=True)) * n
    s2 = (jnp.sum(dl * dl, axis=0, keepdims=True) + jnp.sum(dh * dh, axis=0, keepdims=True)) * n
    var = jnp.maximum(s2 - s1 * s1, 0.0)
    return piv + s1, lax.rsqrt(var + EPS)


def _phi(t):
    return jnp.where(t > 0, t + 1.0, jnp.exp(t))


def _kernel(x_hbm, wq_hbm, wk_hbm, wv_hbm, wo_hbm, beta_hbm, wr_hbm,
            wg_hbm, wu_hbm, wd_hbm, out_hbm,
            x_v, wraw, wtmp, wT, woT, wg_v, wu_v, wd_v, beta_v, wr_v, wr_col,
            k_g, pkT_g, qT_g, pqT_g, vT_g, p_buf, oT, am, MT, grep, omg,
            h_v, h2_v, patch_v, oslow, rb_ref, ib_ref, xe_v, ib_s,
            sem_x, sem_w, sem_f, sem_o, sem_p, sem_s):
    def x_copy(s):
        return pltpu.make_async_copy(x_hbm.at[:, pl.ds(pl.multiple_of(s * L, L), L)], x_v.at[s], sem_x.at[s])

    def w_copy(i):
        src = (wq_hbm, wk_hbm, wv_hbm, wo_hbm)[i]
        return pltpu.make_async_copy(src, wraw.at[i, pl.ds(0, D), :], sem_w.at[i])

    def s_copy(i):
        src, dst = ((beta_hbm, beta_v), (wr_hbm, wr_v))[i]
        return pltpu.make_async_copy(src, dst, sem_s.at[i])

    def f_copy(i):
        src, dst = ((wg_hbm, wg_v), (wu_hbm, wu_v), (wd_hbm, wd_v))[i]
        return pltpu.make_async_copy(src, dst, sem_f.at[i])

    def o_copy(s):
        return pltpu.make_async_copy(h2_v.at[s], out_hbm.at[:, pl.ds(pl.multiple_of(s * L, L), L)], sem_o.at[s])

    wraw[:, pl.ds(D, DP - D), :] = jnp.zeros((4, DP - D, D), BF16)
    w_copy(0).start()
    x_copy(0).start()
    w_copy(1).start()
    w_copy(2).start()
    s_copy(0).start()
    s_copy(1).start()
    w_copy(3).start()

    zi = jnp.zeros((64 - LAST_ROWS // 2, L), I32)
    for ref in (qT_g, pqT_g, pkT_g):
        ref[QV_ROWS // 2:, :] = zi
    vT_g[QV_ROWS:, :] = jnp.zeros((DP - QV_ROWS, L), F32)
    k_g[:, QV_ROWS:] = jnp.zeros((L // 2, DP - QV_ROWS), I32)
    ib_s[0] = 0
    MT[...] = jnp.zeros(MT.shape, F32)
    am[NG - 1] = jnp.zeros((128, L), F32)
    rb_ref[...] = jnp.full((8, L), -jnp.inf, F32)
    ib_ref[...] = jnp.zeros((8, L), I32)

    def windows(src, dst, rows):
        keep = _iota((rows // 2, 128), 1) < HPG * DH
        for g in range(NG - 1):
            w = _pk(src[0:rows, HPG * DH * g: HPG * DH * g + 128])
            dst[0:rows // 2, 128 * g: 128 * (g + 1)] = jnp.where(keep, w, 0)
        dst[0:rows // 2, 512:640] = jnp.zeros((rows // 2, 128), I32)
        dst[0:rows // 2, 512:512 + 72] = _pk(src[0:rows, 504:576])

    for i in range(3):
        w_copy(i).wait()
        windows(wraw.at[i], wtmp, DP)
        ws = -jnp.sum(_f32(wtmp[0:D // 2, :]), axis=0, keepdims=True)
        wh = ws.astype(BF16).astype(F32)
        r16 = _iota((16, DP), 0)
        ext = jnp.where(r16 < 2, wh, jnp.where(r16 == 2, ws - wh, 0.0))
        wtmp[D // 2:D // 2 + 8, :] = _pk(ext.astype(BF16))
        wt = _up(wtmp[...]).T
        wT[_blk(i, QV_ROWS // 2), :] = _pk(wt[0:QV_ROWS, :])
    w_copy(3).wait()
    wtmp[:, 0:D] = _pk(wraw[3])
    wtmp[:, D:DP] = jnp.zeros((DP // 2, DP - D), I32)
    wraw[0, :, :] = _up(wtmp[...]).T[:, 0:D]
    windows(wraw.at[0], woT, D)

    for s in range(1, NSEG):
        x_copy(s).start()
    for i in range(3):
        f_copy(i).start()

    s_copy(0).wait()
    s_copy(1).wait()
    beta = beta_v[...].reshape(1, H).astype(F32)
    gate = jax.nn.sigmoid(beta)
    gate = jnp.concatenate([gate, jnp.zeros((1, 128 - H), F32)], axis=1)
    lane = _iota((128, 128), 1)
    row = _iota((128, 128), 0)
    lane8 = _iota((8, 128), 1)
    row8 = _iota((8, 128), 0)
    for g in range(NG):
        hid = HPG * g + row // DH
        sel = (lane == hid) & (row < _heads_in(g) * DH)
        gcol = jnp.sum(jnp.where(sel, jnp.broadcast_to(gate, (128, 128)), 0.0), axis=1, keepdims=True)
        grep[g] = jnp.broadcast_to(gcol, (128, 128))
        sel8 = (lane8 == HPG * g + row8) & (row8 < _heads_in(g))
        g8 = jnp.sum(jnp.where(sel8, jnp.broadcast_to(gate, (8, 128)), 0.0), axis=1, keepdims=True)
        omg[g] = jnp.broadcast_to(1.0 - g8, (8, 128))
    wr = wr_v[...].reshape(1, D).astype(F32)
    wr = jnp.concatenate([wr, jnp.zeros((1, DP - D), F32)], axis=1)
    wr_col[...] = jnp.broadcast_to(wr, (128, DP)).T

    r128 = _iota((128, 128), 0)
    c128 = _iota((128, 128), 1)
    mrow = _iota((MROWS, 128), 0)
    mlane = _iota((MROWS, 128), 1)
    mhead = jnp.where(mrow < 128, mrow // DH, mrow - 128)
    mmask = (mhead == mlane // DH) & (mlane < HPG * DH) & ((mrow < HPG * DH) | (mrow >= 128))
    ones8 = jnp.ones((8, L), F32)
    kp = 2 * _iota((64, 128), 0)
    qc = _iota((64, 128), 1)
    causal = (jnp.where(kp <= qc, 0x0000FFFF, 0) | jnp.where(kp + 1 <= qc, jnp.int32(-65536), 0))

    def head_window(j):
        return (DH * j // 8) * 8

    def ones_row(j):
        return 0 if DH * j - head_window(j) == 6 else 23

    def ln_in(s):
        rss = []
        for c in range(L // 128):
            cs = slice(128 * c, 128 * (c + 1))
            m, rs = _ln_stats(_pk(x_v[s, :, cs]))
            mh = m.astype(BF16).astype(F32)
            mw = pltpu.bitcast((m - mh).astype(BF16).astype(F32), I32)
            mhw = pltpu.bitcast(mh, I32)
            w0 = mw | lax.shift_right_logical(mhw, 16)
            w1 = lax.shift_right_logical(mhw, 16)
            r8 = _iota((8, 128), 0)
            xe_v[:, cs] = jnp.where(r8 == 0, w0, jnp.where(r8 == 1, w1, 0))
            rss.append(rs)
        return jnp.concatenate(rss, axis=1)

    def proj(i, s):
        xr = _up(jnp.concatenate([_pk(x_v[s]), xe_v[...]], axis=0))
        return lax.dot_general(_up(wT[_blk(i, QV_ROWS // 2), 0:D + 16]), xr,
                               (((1,), (0,)), ((), ())),
                               preferred_element_type=F32)

    def out_proj_post(s):
        for c in range(L // 128):
            cs = slice(128 * c, 128 * (c + 1))
            ot = _up(jnp.concatenate([_unfold(oT, 4 * g + c, 32) for g in range(NG)], axis=0))
            hf = jnp.concatenate(
                [x_v[s, HD * u:HD * (u + 1), cs].astype(F32)
                 + jnp.dot(_up(woT[HD // 2 * u:HD // 2 * (u + 1), :]), ot, preferred_element_type=F32)
                 for u in range(2)], axis=1)
            h_v[_blk(4 * s + c, D // 4), :] = _pk(hf.astype(BF16))
            hw = _unfold(h_v, 4 * s + c + zero, D // 4)
            m, rs = _ln_stats(hw)
            hf = _f32(hw)
            hn = (hf - m) * rs
            h2_v[s, :, cs] = (hf + hn).astype(BF16)
            r = jnp.broadcast_to(jnp.sum(hn * wr_col[0:D, :], axis=0, keepdims=True), (8, 128))
            best = rb_ref[:, cs]
            upd = r > best
            rb_ref[:, cs] = jnp.where(upd, r, best)
            ib_ref[:, cs] = jnp.where(upd, lane8 + (s * L + 128 * c), ib_ref[:, cs])

    def seg_body(s):
        rs = ln_in(s)
        q = proj(0, s) * rs
        qmax = jnp.max(jnp.abs(q))
        qT_g[0:QV_ROWS // 2, :] = _pk((q * QSCALE).astype(BF16))
        if True:
            pqT_g[0:QV_ROWS // 2, :] = _pk(_phi(q).astype(BF16))
        k = proj(1, s) * rs
        kmax = jnp.max(jnp.abs(k))
        k_g[:, 0:QV_ROWS] = _pk(k.astype(BF16).T)
        if True:
            pkT_g[0:QV_ROWS // 2, :] = _pk(_phi(k).astype(BF16))
        v = proj(2, s) * rs
        vmax = jnp.max(jnp.abs(v))
        vT_g[0:QV_ROWS, :] = v
        safe = (qmax * kmax * (DH * QSCALE * 1.02) <= SAFE_BOUND) & (vmax <= V_BOUND)

        for g in range(NG):
            _group(g, 1)

        @pl.when(jnp.logical_not(safe))
        def _():
            _slow_attention()

        @pl.when(s > 0)
        def _():
            o_copy(s - 1).start()

        @pl.when(s + 1 < NSEG)
        def _():
            x_copy(s + 1).wait()
        out_proj_post(s)

    def _group(g, s):
        nh = _heads_in(g)
        g2 = slice(64 * g, 64 * (g + 1))
        mr = -(-nh * DH // 8) * 8
        mt = MT[g] if s > 0 else None
        if s > 0:
            lhs = jnp.concatenate([mt[0:mr] * grep[g, 0:mr], mt[128:MROWS]], axis=0)
            nd = jnp.dot(lhs, _up(pqT_g[g2, :]), preferred_element_type=F32)
            rden = 1.0 / (nd[mr:mr + 8] + 1e-06)
            for r in range(mr // 8):
                lo, hi = 8 * r, 8 * r + 8
                h0, h1 = lo // DH, min((hi - 1) // DH, HPG - 1)
                rd = jnp.broadcast_to(rden[h0:h0 + 1], (8, L))
                if h1 != h0:
                    rd = jnp.where(_iota((8, L), 0) + lo < DH * h1, rd,
                                   jnp.broadcast_to(rden[h1:h1 + 1], (8, L)))
                am[g, lo:hi, :] = nd[lo:hi] * rd
        else:
            am[g] = jnp.zeros((128, L), F32)
        if s < NSEG - 1:
            lhs = jnp.concatenate([vT_g[128 * g:128 * g + mr, :], ones8], axis=0)
            upd = lax.dot_general(lhs, _up(pkT_g[g2, :]), (((1,), (1,)), ((), ())),
                                  preferred_element_type=F32)
            MT[g, 0:mr] = mt[0:mr] + jnp.where(mmask[0:mr], upd[0:mr], 0.0)
            MT[g, 128:MROWS] = mt[128:MROWS] + jnp.where(mmask[128:MROWS], upd[mr:mr + 8], 0.0)

        def qk(qb, slot):
            nk = (qb + 1) * 128
            qt = qT_g[g2, qb * 128:(qb + 1) * 128]
            rr = _iota((64, 128), 0)
            qm = _up(jnp.concatenate(
                [jnp.where((rr >= 9 * j) & (rr < 9 * j + 9), qt, 0)
                 for j in range(nh)], axis=1))
            sc = jnp.dot(_up(k_g[0:nk // 2, 128 * g:128 * (g + 1)]), qm, preferred_element_type=F32)
            p_buf[256 * slot:256 * slot + nk // 2, 0:nh * 128] = _pk(jnp.exp2(sc).astype(BF16))

        def pv(qb, slot):
            nk = (qb + 1) * 128
            vals = []
            for j in range(nh):
                a2 = 128 * g + head_window(j)
                vw = jnp.where(_iota((24, nk), 0) == ones_row(j), 1.0, vT_g[a2:a2 + 24, 0:nk])
                js = slice(j * 128, (j + 1) * 128)
                p0 = 256 * slot
                pw = p_buf[p0 + (nk - 128) // 2:p0 + nk // 2, js] & causal
                if nk > 128:
                    pw = jnp.concatenate([p_buf[p0:p0 + (nk - 128) // 2, js], pw], axis=0)
                acc = jnp.dot(vw, _up(pw), preferred_element_type=F32)
                rd = omg[g, j:j + 1, :] / acc[ones_row(j):ones_row(j) + 1]
                vals.append((acc, jnp.broadcast_to(rd, (8, 128))))
            rows = []
            for r in range(16):
                lo, hi = 8 * r, 8 * r + 8
                h0, h1 = lo // DH, (hi - 1) // DH
                val = am[g, lo:hi, qb * 128:(qb + 1) * 128] if lo < mr else None
                if h0 < nh:
                    a0 = head_window(h0)
                    d = vals[h0][0][lo - a0:hi - a0] * vals[h0][1]
                    if h1 != h0:
                        if h1 < nh:
                            a1 = head_window(h1)
                            d1 = vals[h1][0][lo - a1:hi - a1] * vals[h1][1]
                        else:
                            d1 = jnp.zeros((8, 128), F32)
                        d = jnp.where(row8 + lo < DH * h1, d, d1)
                    val = d if val is None else val + d
                elif val is None:
                    val = jnp.zeros((8, 128), F32)
                rows.append(val)
            oT[_blk(4 * g + qb, 32), :] = _pk(jnp.concatenate(
                [jnp.concatenate(rows[:8], axis=0), jnp.concatenate(rows[8:], axis=0)],
                axis=1).astype(BF16))

        order = (3, 2, 1, 0)
        for i, qb in enumerate(order):
            qk(qb, i % 2)
            if i > 0:
                pv(order[i - 1], (i - 1) % 2)
        pv(order[-1], (len(order) - 1) % 2)

    def _slow_attention():
        def g_body(g, c):
            oslow[...] = am[g]

            def j_body(j, c2):
                a = pl.multiple_of((DH * j // 16) * 16, 16)
                lo = DH * j

                def q_body(qb, c3):
                    q0 = pl.multiple_of(qb * 128, 128)
                    g64 = pl.multiple_of(g * 64, 64)
                    qt = _up(qT_g[pl.ds(g64, 64), pl.ds(q0, 128)])
                    qm = jnp.where((r128 >= lo) & (r128 < lo + DH), qt, jnp.zeros_like(qt))
                    sc = jnp.dot(_up(k_g[:, pl.ds(pl.multiple_of(g * 128, 128), 128)]), qm,
                                 preferred_element_type=F32)
                    ok = _iota((L, 128), 0) <= _iota((L, 128), 1) + q0
                    sc = jnp.where(ok, sc, -jnp.inf)
                    mx = jnp.max(sc, axis=0, keepdims=True)
                    p = jnp.exp2(sc - mx).astype(BF16)
                    vw = vT_g[pl.ds(pl.multiple_of(2 * g64 + a, 16), 32), :]
                    vw = jnp.where(_iota((32, L), 0) == 31, 1.0, vw)
                    acc = jnp.dot(vw, p, preferred_element_type=F32)
                    rr = _iota((32, 128), 0) + a
                    keep = (rr >= lo) & (rr < lo + DH)
                    gj = grep[g, pl.ds(a, 32), :]
                    val = acc * ((1.0 - gj) / acc[31:32])
                    cur = oslow[pl.ds(a, 32), pl.ds(q0, 128)]
                    oslow[pl.ds(a, 32), pl.ds(q0, 128)] = jnp.where(keep, cur + val, cur)
                    return c3
                return lax.fori_loop(0, 4, q_body, c2)
            lax.fori_loop(0, HPG, j_body, 0)
            for qb in range(4):
                qs = slice(128 * qb, 128 * (qb + 1))
                oT[_blk(4 * g + qb, 32), :] = _pk(
                    jnp.concatenate([oslow[0:64, qs], oslow[64:128, qs]], axis=1).astype(BF16))
            return c
        lax.fori_loop(0, NG, g_body, 0)

    zero = ib_s[0]
    x_copy(0).wait()
    lax.fori_loop(0, NSEG, lambda s, c: (seg_body(s), c)[1], 0)

    o_copy(NSEG - 1).start()
    rb = rb_ref[...]
    rmax = jnp.max(rb)
    idx = jnp.min(jnp.where(rb == rmax, ib_ref[...], SEQ))
    idx = jnp.clip(idx, 0, SEQ - 1)
    hw = _unfold(h_v, idx // 128, D // 4)
    m, rs = _ln_stats(hw)
    hf = _up(hw).astype(F32)
    hn = ((hf - m) * rs).astype(BF16)
    hrow = jnp.concatenate([hn, jnp.zeros((DP - D, 128), BF16)], axis=0).T
    pick_r = _iota((128, DP), 0) == (idx % 128)
    xs = jnp.sum(jnp.where(pick_r, hrow.astype(F32), 0.0), axis=0, keepdims=True)
    xs = jnp.broadcast_to(xs[:, 0:D], (16, D)).astype(BF16)
    for i in range(3):
        f_copy(i).wait()
    gt = jnp.dot(xs, wg_v[...], preferred_element_type=F32)[0:8]
    up = jnp.dot(xs, wu_v[...], preferred_element_type=F32)[0:8]
    act = (gt * jax.nn.sigmoid(gt) * up)
    act = jnp.concatenate([act, act], axis=0).astype(BF16)
    y = lax.dot_general(act, wd_v[...], (((1,), (1,)), ((), ())),
                        preferred_element_type=F32)[0:1]
    y = y * jax.nn.sigmoid(jnp.full((1, D), rmax, F32))
    y = jnp.concatenate([y, jnp.zeros((1, DP - D), F32)], axis=1)
    ycol = jnp.broadcast_to(y, (128, DP)).T[0:D]
    hn = hn.astype(F32)
    new = (hf + (hn + ycol).astype(BF16).astype(F32)).astype(BF16)
    old = (hf + hn).astype(BF16)
    patch_v[...] = jnp.where(_iota((D, 128), 1) == (idx % 128), new, old)
    for s in range(NSEG):
        o_copy(s).wait()
    p0 = pl.multiple_of((idx // 128) * 128, 128)
    cp = pltpu.make_async_copy(patch_v, out_hbm.at[:, pl.ds(p0, 128)], sem_p)
    cp.start()
    cp.wait()


@jax.jit
def pallas_sequential_preLN__memory_aug_infini_attn__moe_arch_mod__prompt_kernel(
    A_x: jax.Array,
    A_wq: jax.Array,
    A_wk: jax.Array,
    A_wv: jax.Array,
    A_wo: jax.Array,
    A_beta: jax.Array,
    B_x: jax.Array,
    B_w_r: jax.Array,
    B_w_gate: jax.Array,
    B_w_up: jax.Array,
    B_w_down: jax.Array,
):
    del B_x
    hbm = pl.BlockSpec(memory_space=pltpu.HBM)
    VM = pltpu.VMEM
    outT = pl.pallas_call(
        _kernel,
        out_shape=jax.ShapeDtypeStruct((D, SEQ), BF16),
        in_specs=[hbm] * 10,
        out_specs=hbm,
        scratch_shapes=[
            VM((NSEG, D, L), BF16),
            VM((4, DP, D), BF16),
            VM((DP // 2, DP), I32),
            VM((3 * QV_ROWS // 2, DP), I32),
            VM((D // 2, DP), I32),
            VM((D, FF), BF16),
            VM((D, FF), BF16),
            VM((D, FF), BF16),
            VM((H,), BF16),
            VM((D,), BF16),
            VM((DP, 128), F32),
            VM((L // 2, DP), I32),
            VM((NG * 64, L), I32),
            VM((NG * 64, L), I32),
            VM((NG * 64, L), I32),
            VM((DP, L), F32),
            VM((L, HPG * 128), I32),
            VM((NG * 4 * 32, 256), I32),
            VM((NG, 128, L), F32),
            VM((NG, MROWS, 128), F32),
            VM((NG, 128, 128), F32),
            VM((NG, 8, 128), F32),
            VM((NSEG * D, 256), I32),
            VM((NSEG, D, L), BF16),
            VM((D, 128), BF16),
            VM((128, L), F32),
            VM((8, L), F32),
            VM((8, L), I32),
            VM((8, L), I32),
            pltpu.SMEM((1,), I32),
            pltpu.SemaphoreType.DMA((NSEG,)),
            pltpu.SemaphoreType.DMA((4,)),
            pltpu.SemaphoreType.DMA((3,)),
            pltpu.SemaphoreType.DMA((NSEG,)),
            pltpu.SemaphoreType.DMA(()),
            pltpu.SemaphoreType.DMA((2,)),
        ],
        compiler_params=pltpu.CompilerParams(vmem_limit_bytes=64 * 1024 * 1024),
    )(A_x.reshape(SEQ, D).T, A_wq, A_wk, A_wv, A_wo, A_beta, B_w_r,
      B_w_gate, B_w_up, B_w_down.T)
    return outT.T.reshape(1, SEQ, D)
```

```python
import functools

import jax
import jax.numpy as jnp
import numpy as np
from jax import lax
import jax.experimental.pallas as pl
import jax.experimental.pallas.tpu as pltpu

F32 = jnp.float32
BF16 = jnp.bfloat16
I32 = jnp.int32

SEQ = 2048
D = 576
DP = 640
H = 32
DH = 18
NSEG = 4
L = 512
FF = 4608
NG = 5
HPG = 7
LAST_ROWS = 80
QV_ROWS = 4 * 128 + LAST_ROWS
EPS = 1e-05
LOG2E = 1.4426950408889634
QSCALE = float(DH ** -0.5) * LOG2E
SAFE_BOUND = 40.0
V_BOUND = 2.0 ** 40
HD = D // 2
MROWS = 136


def _heads_in(g):
    return min(HPG, H - HPG * g)


def _iota(shape, dim):
    return lax.broadcasted_iota(I32, shape, dim)


def _pk(v):
    return pltpu.bitcast(v, I32)


def _up(w):
    return pltpu.bitcast(w, BF16)


def _blk(i, n):
    if isinstance(i, int):
        return slice(i * n, (i + 1) * n)
    return pl.ds(pl.multiple_of(i * n, 8), n)


def _unfold(ref, i, n):
    return jnp.concatenate([ref[_blk(i, n), 0:128], ref[_blk(i, n), 128:256]], axis=0)


def _f32(w):
    return _up(w).astype(F32)


def _ln_stats(w):
    lo = pltpu.bitcast(w << 16, F32)
    hi = pltpu.bitcast(w & jnp.int32(-65536), F32)
    piv = lo[0:1]
    dl = lo - piv
    dh = hi - piv
    n = 1.0 / (2 * w.shape[0])
    s1 = (jnp.sum(dl, axis=0, keepdims=True) + jnp.sum(dh, axis=0, keepdims=True)) * n
    s2 = (jnp.sum(dl * dl, axis=0, keepdims=True) + jnp.sum(dh * dh, axis=0, keepdims=True)) * n
    var = jnp.maximum(s2 - s1 * s1, 0.0)
    return piv + s1, lax.rsqrt(var + EPS)


def _phi(t):
    return jnp.where(t > 0, t + 1.0, jnp.exp(t))


def _kernel(x_hbm, wq_hbm, wk_hbm, wv_hbm, wo_hbm, beta_hbm, wr_hbm,
            wg_hbm, wu_hbm, wd_hbm, out_hbm,
            x_v, wraw, wT, woT, wg_v, wu_v, wd_v, beta_v, wr_v, wr_col,
            k_g, pkT_g, qT_g, pqT_g, vT_g, p_buf, oT, am, MT, grep, omg,
            h_v, h2_v, patch_v, oslow, rb_ref, ib_ref, xe_v, ib_s, wdT,
            sem_x, sem_w, sem_f, sem_o, sem_p, sem_s):
    def x_copy(s):
        return pltpu.make_async_copy(x_hbm.at[:, pl.ds(pl.multiple_of(s * L, L), L)], x_v.at[s], sem_x.at[s])

    def w_copy(i):
        src = (wq_hbm, wk_hbm, wv_hbm, wo_hbm)[i]
        return pltpu.make_async_copy(src, wraw.at[i, pl.ds(0, D), :], sem_w.at[i])

    def s_copy(i):
        src, dst = ((beta_hbm, beta_v), (wr_hbm, wr_v))[i]
        return pltpu.make_async_copy(src, dst, sem_s.at[i])

    def f_copy(i):
        src, dst = ((wg_hbm, wg_v), (wu_hbm, wu_v), (wd_hbm, wd_v.at[:, pl.ds(0, FF)]))[i]
        return pltpu.make_async_copy(src, dst, sem_f.at[i])

    def o_copy(s):
        return pltpu.make_async_copy(h2_v.at[s], out_hbm.at[:, pl.ds(pl.multiple_of(s * L, L), L)], sem_o.at[s])

    wraw[:, pl.ds(D, DP - D), :] = jnp.zeros((4, DP - D, D), BF16)
    w_copy(0).start()
    w_copy(1).start()
    s_copy(0).start()
    s_copy(1).start()

    zi = jnp.zeros((64 - LAST_ROWS // 2, L), I32)
    for ref in (qT_g, pqT_g, pkT_g):
        ref[QV_ROWS // 2:, :] = zi
    vT_g[QV_ROWS:, :] = jnp.zeros((DP - QV_ROWS, L), F32)
    k_g[:, QV_ROWS:] = jnp.zeros((L // 2, DP - QV_ROWS), I32)
    ib_s[0] = 0
    MT[...] = jnp.zeros(MT.shape, F32)
    am[NG - 1] = jnp.zeros((128, L), F32)
    rb_ref[...] = jnp.full((8, L), -jnp.inf, F32)
    ib_ref[...] = jnp.zeros((8, L), I32)

    def respace(w, last):
        keep = _iota((64, w.shape[1]), 0) < HPG * DH // 2
        out = [jnp.where(keep, w[63 * g:63 * g + 64], 0) for g in range(NG - 1)]
        out += [w[252:288], jnp.zeros((last - 36, w.shape[1]), I32)]
        return jnp.concatenate(out, axis=0)

    for i in range(3):
        w_copy(i).wait()
        if i < 2:
            w_copy(i + 2).start()
        else:
            x_copy(0).start()
        ws = -jnp.sum(wraw[i, 0:D, :].astype(F32), axis=0, keepdims=True)
        wh = ws.astype(BF16).astype(F32)
        r16 = _iota((16, D), 0)
        ext = jnp.where(r16 < 2, wh, jnp.where(r16 == 2, ws - wh, 0.0))
        wraw[i, D:D + 16, :] = ext.astype(BF16)
        wT[_blk(i, QV_ROWS // 2), :] = respace(_pk(wraw[i].T), LAST_ROWS // 2)
    w_copy(3).wait()
    s_copy(0).wait()
    s_copy(1).wait()
    woT[...] = _pk(_up(respace(_pk(wraw[3, 0:D, :]), 64)).T)

    for s in range(1, NSEG):
        x_copy(s).start()
    for i in (2, 0, 1):
        f_copy(i).start()

    beta = beta_v[...].reshape(1, H).astype(F32)
    gate = jax.nn.sigmoid(beta)
    gate = jnp.concatenate([gate, jnp.zeros((1, 128 - H), F32)], axis=1)
    lane = _iota((128, 128), 1)
    row = _iota((128, 128), 0)
    lane8 = _iota((8, 128), 1)
    row8 = _iota((8, 128), 0)
    for g in range(NG):
        hid = HPG * g + row // DH
        sel = (lane == hid) & (row < _heads_in(g) * DH)
        gcol = jnp.sum(jnp.where(sel, jnp.broadcast_to(gate, (128, 128)), 0.0), axis=1, keepdims=True)
        grep[g] = jnp.broadcast_to(gcol, (128, 128))
        sel8 = (lane8 == HPG * g + row8) & (row8 < _heads_in(g))
        g8 = jnp.sum(jnp.where(sel8, jnp.broadcast_to(gate, (8, 128)), 0.0), axis=1, keepdims=True)
        omg[g] = jnp.broadcast_to(1.0 - g8, (8, 128))
    wr = wr_v[...].reshape(1, D).astype(F32)
    wr = jnp.concatenate([wr, jnp.zeros((1, DP - D), F32)], axis=1)
    wr_col[...] = jnp.broadcast_to(wr, (128, DP)).T

    r128 = _iota((128, 128), 0)
    c128 = _iota((128, 128), 1)
    mrow = _iota((MROWS, 128), 0)
    mlane = _iota((MROWS, 128), 1)
    mhead = jnp.where(mrow < 128, mrow // DH, mrow - 128)
    mmask = (mhead == mlane // DH) & (mlane < HPG * DH) & ((mrow < HPG * DH) | (mrow >= 128))
    ones8 = jnp.ones((8, L), F32)
    kp = 2 * _iota((64, 128), 0)
    qc = _iota((64, 128), 1)
    causal = (jnp.where(kp <= qc, 0x0000FFFF, 0) | jnp.where(kp + 1 <= qc, jnp.int32(-65536), 0))

    def head_window(j):
        return (DH * j // 8) * 8

    def ones_row(j):
        return 0 if DH * j - head_window(j) == 6 else 23

    def ln_in(s):
        rss = []
        for c in range(L // 128):
            cs = slice(128 * c, 128 * (c + 1))
            m, rs = _ln_stats(_pk(x_v[s, :, cs]))
            mh = m.astype(BF16).astype(F32)
            mw = pltpu.bitcast((m - mh).astype(BF16).astype(F32), I32)
            mhw = pltpu.bitcast(mh, I32)
            w0 = mw | lax.shift_right_logical(mhw, 16)
            w1 = lax.shift_right_logical(mhw, 16)
            r8 = _iota((8, 128), 0)
            xe_v[:, cs] = jnp.where(r8 == 0, w0, jnp.where(r8 == 1, w1, 0))
            rss.append(rs)
        return jnp.concatenate(rss, axis=1)

    def proj(i, s):
        xr = _up(jnp.concatenate([_pk(x_v[s]), xe_v[...]], axis=0))
        return lax.dot_general(_up(wT[_blk(i, QV_ROWS // 2), 0:D + 16]), xr,
                               (((1,), (0,)), ((), ())),
                               preferred_element_type=F32)

    def out_proj_post(s):
        for c in range(L // 128):
            cs = slice(128 * c, 128 * (c + 1))
            ot = _up(jnp.concatenate([_unfold(oT, 4 * g + c, 32) for g in range(NG)], axis=0))
            hf = jnp.concatenate(
                [x_v[s, HD * u:HD * (u + 1), cs].astype(F32)
                 + jnp.dot(_up(woT[HD // 2 * u:HD // 2 * (u + 1), :]), ot, preferred_element_type=F32)
                 for u in range(2)], axis=1)
            h_v[_blk(4 * s + c, D // 4), :] = _pk(hf.astype(BF16))
            hw = _unfold(h_v, 4 * s + c + zero, D // 4)
            m, rs = _ln_stats(hw)
            hf = _f32(hw)
            hn = (hf - m) * rs
            h2_v[s, :, cs] = (hf + hn).astype(BF16)
            r = jnp.broadcast_to(jnp.sum(hn * wr_col[0:D, :], axis=0, keepdims=True), (8, 128))
            best = rb_ref[:, cs]
            upd = r > best
            rb_ref[:, cs] = jnp.where(upd, r, best)
            ib_ref[:, cs] = jnp.where(upd, lane8 + (s * L + 128 * c), ib_ref[:, cs])

    def seg_body(s):
        rs = ln_in(s)
        q = proj(0, s) * rs
        qmax = jnp.max(jnp.abs(q))
        qT_g[0:QV_ROWS // 2, :] = _pk((q * QSCALE).astype(BF16))
        if True:
            pqT_g[0:QV_ROWS // 2, :] = _pk(_phi(q).astype(BF16))
        k = proj(1, s) * rs
        kmax = jnp.max(jnp.abs(k))
        k_g[:, 0:QV_ROWS] = _pk(k.astype(BF16).T)
        if True:
            pkT_g[0:QV_ROWS // 2, :] = _pk(_phi(k).astype(BF16))
        v = proj(2, s) * rs
        vmax = jnp.max(jnp.abs(v))
        vT_g[0:QV_ROWS, :] = v
        safe = (qmax * kmax * (DH * QSCALE * 1.02) <= SAFE_BOUND) & (vmax <= V_BOUND)

        f0 = jnp.where(s > 0, s - 1, 3) * (FF // 3)
        for g in range(NG):
            for t in range(3 * g, min(3 * g + 3, 12)):
                fc = pl.multiple_of(f0 + 128 * t, 128)
                wdT[pl.ds(pl.multiple_of(fc // 2, 64), 64), 0:D] = _pk(wd_v[:, pl.ds(fc, 128)].T)
            _group(g, 1)

        @pl.when(jnp.logical_not(safe))
        def _():
            _slow_attention()

        @pl.when(s > 0)
        def _():
            o_copy(s - 1).start()

        @pl.when(s == 0)
        def _():
            f_copy(2).wait()

        @pl.when(s + 1 < NSEG)
        def _():
            x_copy(s + 1).wait()
        out_proj_post(s)

    def _group(g, s):
        nh = _heads_in(g)
        g2 = slice(64 * g, 64 * (g + 1))
        mr = -(-nh * DH // 8) * 8
        mt = MT[g] if s > 0 else None
        if s > 0:
            lhs = jnp.concatenate([mt[0:mr] * grep[g, 0:mr], mt[128:MROWS]], axis=0)
            nd = jnp.dot(lhs, _up(pqT_g[g2, :]), preferred_element_type=F32)
            rden = 1.0 / (nd[mr:mr + 8] + 1e-06)
            for r in range(mr // 8):
                lo, hi = 8 * r, 8 * r + 8
                h0, h1 = lo // DH, min((hi - 1) // DH, HPG - 1)
                rd = jnp.broadcast_to(rden[h0:h0 + 1], (8, L))
                if h1 != h0:
                    rd = jnp.where(_iota((8, L), 0) + lo < DH * h1, rd,
                                   jnp.broadcast_to(rden[h1:h1 + 1], (8, L)))
                am[g, lo:hi, :] = nd[lo:hi] * rd
        else:
            am[g] = jnp.zeros((128, L), F32)
        if s < NSEG - 1:
            lhs = jnp.concatenate([vT_g[128 * g:128 * g + mr, :], ones8], axis=0)
            upd = lax.dot_general(lhs, _up(pkT_g[g2, :]), (((1,), (1,)), ((), ())),
                                  preferred_element_type=F32)
            MT[g, 0:mr] = mt[0:mr] + jnp.where(mmask[0:mr], upd[0:mr], 0.0)
            MT[g, 128:MROWS] = mt[128:MROWS] + jnp.where(mmask[128:MROWS], upd[mr:mr + 8], 0.0)

        def qk(qb, slot):
            nk = (qb + 1) * 128
            qt = qT_g[g2, qb * 128:(qb + 1) * 128]
            rr = _iota((64, 128), 0)
            qm = _up(jnp.concatenate(
                [jnp.where((rr >= 9 * j) & (rr < 9 * j + 9), qt, 0)
                 for j in range(nh)], axis=1))
            sc = jnp.dot(_up(k_g[0:nk // 2, 128 * g:128 * (g + 1)]), qm, preferred_element_type=F32)
            p_buf[256 * slot:256 * slot + nk // 2, 0:nh * 128] = _pk(jnp.exp2(sc).astype(BF16))

        def pv(qb, slot):
            nk = (qb + 1) * 128
            vals = []
            for j in range(nh):
                a2 = 128 * g + head_window(j)
                vw = jnp.where(_iota((24, nk), 0) == ones_row(j), 1.0, vT_g[a2:a2 + 24, 0:nk])
                js = slice(j * 128, (j + 1) * 128)
                p0 = 256 * slot
                pw = p_buf[p0 + (nk - 128) // 2:p0 + nk // 2, js] & causal
                if nk > 128:
                    pw = jnp.concatenate([p_buf[p0:p0 + (nk - 128) // 2, js], pw], axis=0)
                acc = jnp.dot(vw, _up(pw), preferred_element_type=F32)
                rd = omg[g, j:j + 1, :] / acc[ones_row(j):ones_row(j) + 1]
                vals.append((acc, jnp.broadcast_to(rd, (8, 128))))
            rows = []
            for r in range(16):
                lo, hi = 8 * r, 8 * r + 8
                h0, h1 = lo // DH, (hi - 1) // DH
                val = am[g, lo:hi, qb * 128:(qb + 1) * 128] if lo < mr else None
                if h0 < nh:
                    a0 = head_window(h0)
                    d = vals[h0][0][lo - a0:hi - a0] * vals[h0][1]
                    if h1 != h0:
                        if h1 < nh:
                            a1 = head_window(h1)
                            d1 = vals[h1][0][lo - a1:hi - a1] * vals[h1][1]
                        else:
                            d1 = jnp.zeros((8, 128), F32)
                        d = jnp.where(row8 + lo < DH * h1, d, d1)
                    val = d if val is None else val + d
                elif val is None:
                    val = jnp.zeros((8, 128), F32)
                rows.append(val)
            oT[_blk(4 * g + qb, 32), :] = _pk(jnp.concatenate(
                [jnp.concatenate(rows[:8], axis=0), jnp.concatenate(rows[8:], axis=0)],
                axis=1).astype(BF16))

        order = (3, 2, 1, 0)
        for i, qb in enumerate(order):
            qk(qb, i % 2)
            if i > 0:
                pv(order[i - 1], (i - 1) % 2)
        pv(order[-1], (len(order) - 1) % 2)

    def _slow_attention():
        def g_body(g, c):
            oslow[...] = am[g]

            def j_body(j, c2):
                a = pl.multiple_of((DH * j // 16) * 16, 16)
                lo = DH * j

                def q_body(qb, c3):
                    q0 = pl.multiple_of(qb * 128, 128)
                    g64 = pl.multiple_of(g * 64, 64)
                    qt = _up(qT_g[pl.ds(g64, 64), pl.ds(q0, 128)])
                    qm = jnp.where((r128 >= lo) & (r128 < lo + DH), qt, jnp.zeros_like(qt))
                    sc = jnp.dot(_up(k_g[:, pl.ds(pl.multiple_of(g * 128, 128), 128)]), qm,
                                 preferred_element_type=F32)
                    ok = _iota((L, 128), 0) <= _iota((L, 128), 1) + q0
                    sc = jnp.where(ok, sc, -jnp.inf)
                    mx = jnp.max(sc, axis=0, keepdims=True)
                    p = jnp.exp2(sc - mx).astype(BF16)
                    vw = vT_g[pl.ds(pl.multiple_of(2 * g64 + a, 16), 32), :]
                    vw = jnp.where(_iota((32, L), 0) == 31, 1.0, vw)
                    acc = jnp.dot(vw, p, preferred_element_type=F32)
                    rr = _iota((32, 128), 0) + a
                    keep = (rr >= lo) & (rr < lo + DH)
                    gj = grep[g, pl.ds(a, 32), :]
                    val = acc * ((1.0 - gj) / acc[31:32])
                    cur = oslow[pl.ds(a, 32), pl.ds(q0, 128)]
                    oslow[pl.ds(a, 32), pl.ds(q0, 128)] = jnp.where(keep, cur + val, cur)
                    return c3
                return lax.fori_loop(0, 4, q_body, c2)
            lax.fori_loop(0, HPG, j_body, 0)
            for qb in range(4):
                qs = slice(128 * qb, 128 * (qb + 1))
                oT[_blk(4 * g + qb, 32), :] = _pk(
                    jnp.concatenate([oslow[0:64, qs], oslow[64:128, qs]], axis=1).astype(BF16))
            return c
        lax.fori_loop(0, NG, g_body, 0)

    zero = ib_s[0]
    x_copy(0).wait()
    lax.fori_loop(0, NSEG, lambda s, c: (seg_body(s), c)[1], 0)

    o_copy(NSEG - 1).start()
    rb = rb_ref[...]
    rmax = jnp.max(rb)
    idx = jnp.min(jnp.where(rb == rmax, ib_ref[...], SEQ))
    idx = jnp.clip(idx, 0, SEQ - 1)
    hw = _unfold(h_v, idx // 128, D // 4)
    m, rs = _ln_stats(hw)
    hf = _up(hw).astype(F32)
    hn = ((hf - m) * rs).astype(BF16)
    hrow = jnp.concatenate([hn, jnp.zeros((DP - D, 128), BF16)], axis=0).T
    pick_r = _iota((128, DP), 0) == (idx % 128)
    xs = jnp.sum(jnp.where(pick_r, hrow.astype(F32), 0.0), axis=0, keepdims=True)
    xs = jnp.broadcast_to(xs[:, 0:D], (16, D)).astype(BF16)
    for i in range(2):
        f_copy(i).wait()
    gt = jnp.dot(xs, wg_v[...], preferred_element_type=F32)[0:8]
    up = jnp.dot(xs, wu_v[...], preferred_element_type=F32)[0:8]
    act = (gt * jax.nn.sigmoid(gt) * up)
    act = jnp.concatenate([act, act], axis=0).astype(BF16)
    y = jnp.dot(act, _up(wdT[0:FF // 2, 0:D]), preferred_element_type=F32)[0:1]
    y = y * jax.nn.sigmoid(jnp.full((1, D), rmax, F32))
    y = jnp.concatenate([y, jnp.zeros((1, DP - D), F32)], axis=1)
    ycol = jnp.broadcast_to(y, (128, DP)).T[0:D]
    hn = hn.astype(F32)
    new = (hf + (hn + ycol).astype(BF16).astype(F32)).astype(BF16)
    old = (hf + hn).astype(BF16)
    patch_v[...] = jnp.where(_iota((D, 128), 1) == (idx % 128), new, old)
    for s in range(NSEG):
        o_copy(s).wait()
    p0 = pl.multiple_of((idx // 128) * 128, 128)
    cp = pltpu.make_async_copy(patch_v, out_hbm.at[:, pl.ds(p0, 128)], sem_p)
    cp.start()
    cp.wait()


@jax.jit
def pallas_sequential_preLN__memory_aug_infini_attn__moe_arch_mod__prompt_kernel(
    A_x: jax.Array,
    A_wq: jax.Array,
    A_wk: jax.Array,
    A_wv: jax.Array,
    A_wo: jax.Array,
    A_beta: jax.Array,
    B_x: jax.Array,
    B_w_r: jax.Array,
    B_w_gate: jax.Array,
    B_w_up: jax.Array,
    B_w_down: jax.Array,
):
    del B_x
    hbm = pl.BlockSpec(memory_space=pltpu.HBM)
    VM = pltpu.VMEM
    outT = pl.pallas_call(
        _kernel,
        out_shape=jax.ShapeDtypeStruct((D, SEQ), BF16),
        in_specs=[hbm] * 10,
        out_specs=hbm,
        scratch_shapes=[
            VM((NSEG, D, L), BF16),
            VM((4, DP, D), BF16),
            VM((3 * QV_ROWS // 2, DP), I32),
            VM((D // 2, DP), I32),
            VM((D, FF), BF16),
            VM((D, FF), BF16),
            VM((D, FF + FF // 3), BF16),
            VM((H,), BF16),
            VM((D,), BF16),
            VM((DP, 128), F32),
            VM((L // 2, DP), I32),
            VM((NG * 64, L), I32),
            VM((NG * 64, L), I32),
            VM((NG * 64, L), I32),
            VM((DP, L), F32),
            VM((L, HPG * 128), I32),
            VM((NG * 4 * 32, 256), I32),
            VM((NG, 128, L), F32),
            VM((NG, MROWS, 128), F32),
            VM((NG, 128, 128), F32),
            VM((NG, 8, 128), F32),
            VM((NSEG * D, 256), I32),
            VM((NSEG, D, L), BF16),
            VM((D, 128), BF16),
            VM((128, L), F32),
            VM((8, L), F32),
            VM((8, L), I32),
            VM((8, L), I32),
            pltpu.SMEM((1,), I32),
            VM(((FF + FF // 3) // 2, DP), I32),
            pltpu.SemaphoreType.DMA((NSEG,)),
            pltpu.SemaphoreType.DMA((4,)),
            pltpu.SemaphoreType.DMA((3,)),
            pltpu.SemaphoreType.DMA((NSEG,)),
            pltpu.SemaphoreType.DMA(()),
            pltpu.SemaphoreType.DMA((2,)),
        ],
        compiler_params=pltpu.CompilerParams(vmem_limit_bytes=64 * 1024 * 1024),
    )(A_x.reshape(SEQ, D).T, A_wq, A_wk, A_wv, A_wo, A_beta, B_w_r,
      B_w_gate, B_w_up, B_w_down.T)
    return outT.T.reshape(1, SEQ, D)
```

```python
import jax
import jax.numpy as jnp
from jax import lax
import jax.experimental.pallas as pl
import jax.experimental.pallas.tpu as pltpu

F32 = jnp.float32
BF16 = jnp.bfloat16
I32 = jnp.int32

SEQ = 2048
D = 576
DP = 640
H = 32
DH = 18
NSEG = 4
L = 512
FF = 4608
NG = 5
HPG = 7
LAST_ROWS = 80
QV_ROWS = 4 * 128 + LAST_ROWS
EPS = 1e-05
LOG2E = 1.4426950408889634
QSCALE = float(DH ** -0.5) * LOG2E
SAFE_BOUND = 40.0
V_BOUND = 2.0 ** 40
HD = D // 2
MROWS = 136


def _heads_in(g):
    return min(HPG, H - HPG * g)


def _iota(shape, dim):
    return lax.broadcasted_iota(I32, shape, dim)


def _pk(v):
    return pltpu.bitcast(v, I32)


def _up(w):
    return pltpu.bitcast(w, BF16)


def _blk(i, n):
    if isinstance(i, int):
        return slice(i * n, (i + 1) * n)
    return pl.ds(pl.multiple_of(i * n, 8), n)


def _unfold(ref, i, n):
    return jnp.concatenate([ref[_blk(i, n), 0:128], ref[_blk(i, n), 128:256]], axis=0)


def _f32(w):
    return _up(w).astype(F32)


def _ln_stats(w):
    lo = pltpu.bitcast(w << 16, F32)
    hi = pltpu.bitcast(w & jnp.int32(-65536), F32)
    piv = lo[0:1]
    dl = lo - piv
    dh = hi - piv
    n = 1.0 / (2 * w.shape[0])
    s1 = (jnp.sum(dl, axis=0, keepdims=True) + jnp.sum(dh, axis=0, keepdims=True)) * n
    s2 = (jnp.sum(dl * dl, axis=0, keepdims=True) + jnp.sum(dh * dh, axis=0, keepdims=True)) * n
    var = jnp.maximum(s2 - s1 * s1, 0.0)
    return piv + s1, lax.rsqrt(var + EPS)


def _phi(t):
    return jnp.where(t > 0, t + 1.0, jnp.exp(t))


def _kernel(x_hbm, wq_hbm, wk_hbm, wv_hbm, wo_hbm, beta_hbm, wr_hbm,
            wg_hbm, wu_hbm, wd_hbm, out_hbm,
            x_v, wraw, wT, woT, wg_v, wu_v, wd_v, beta_v, wr_v, wr_col,
            k_g, pkT_g, qT_g, pqT_g, vT_g, p_buf, oT, am, MT, grep, omg,
            h_v, h2_v, patch_v, oslow, rb_ref, ib_ref, xe_v, ib_s, wdT,
            sem_x, sem_w, sem_f, sem_o, sem_p, sem_s):
    def x_copy(s):
        return pltpu.make_async_copy(x_hbm.at[:, pl.ds(pl.multiple_of(s * L, L), L)], x_v.at[s], sem_x.at[s])

    def w_copy(i):
        src = (wq_hbm, wk_hbm, wv_hbm, wo_hbm)[i]
        return pltpu.make_async_copy(src, wraw.at[i, pl.ds(0, D), :], sem_w.at[i])

    def s_copy(i):
        src, dst = ((beta_hbm, beta_v), (wr_hbm, wr_v))[i]
        return pltpu.make_async_copy(src, dst, sem_s.at[i])

    def f_copy(i):
        src, dst = ((wg_hbm, wg_v), (wu_hbm, wu_v), (wd_hbm, wd_v.at[:, pl.ds(0, FF)]))[i]
        return pltpu.make_async_copy(src, dst, sem_f.at[i])

    def o_copy(s):
        return pltpu.make_async_copy(h2_v.at[s], out_hbm.at[:, pl.ds(pl.multiple_of(s * L, L), L)], sem_o.at[s])

    wraw[:, pl.ds(D, DP - D), :] = jnp.zeros((4, DP - D, D), BF16)
    w_copy(0).start()
    w_copy(1).start()
    s_copy(0).start()
    s_copy(1).start()

    zi = jnp.zeros((64 - LAST_ROWS // 2, L), I32)
    for ref in (qT_g, pqT_g, pkT_g):
        ref[QV_ROWS // 2:, :] = zi
    vT_g[QV_ROWS:, :] = jnp.zeros((DP - QV_ROWS, L), F32)
    k_g[:, QV_ROWS:] = jnp.zeros((L // 2, DP - QV_ROWS), I32)
    ib_s[0] = 0
    MT[...] = jnp.zeros(MT.shape, F32)
    am[NG - 1] = jnp.zeros((128, L), F32)
    rb_ref[...] = jnp.full((8, L), -jnp.inf, F32)
    ib_ref[...] = jnp.zeros((8, L), I32)

    def respace(w, last):
        keep = _iota((64, w.shape[1]), 0) < HPG * DH // 2
        out = [jnp.where(keep, w[63 * g:63 * g + 64], 0) for g in range(NG - 1)]
        out += [w[252:288], jnp.zeros((last - 36, w.shape[1]), I32)]
        return jnp.concatenate(out, axis=0)

    for i in range(3):
        w_copy(i).wait()
        if i < 2:
            w_copy(i + 2).start()
        else:
            x_copy(0).start()
        ws = -jnp.sum(wraw[i, 0:D, :].astype(F32), axis=0, keepdims=True)
        wh = ws.astype(BF16).astype(F32)
        r16 = _iota((16, D), 0)
        ext = jnp.where(r16 < 2, wh, jnp.where(r16 == 2, ws - wh, 0.0))
        wraw[i, D:D + 16, :] = ext.astype(BF16)
        wT[_blk(i, QV_ROWS // 2), :] = respace(_pk(wraw[i].T), LAST_ROWS // 2)
    w_copy(3).wait()
    s_copy(0).wait()
    s_copy(1).wait()
    woT[...] = _pk(_up(respace(_pk(wraw[3, 0:D, :]), 64)).T)

    for s in range(1, NSEG):
        x_copy(s).start()
    for i in (2, 0, 1):
        f_copy(i).start()

    beta = beta_v[...].reshape(1, H).astype(F32)
    gate = jax.nn.sigmoid(beta)
    gate = jnp.concatenate([gate, jnp.zeros((1, 128 - H), F32)], axis=1)
    lane = _iota((128, 128), 1)
    row = _iota((128, 128), 0)
    lane8 = _iota((8, 128), 1)
    row8 = _iota((8, 128), 0)
    for g in range(NG):
        hid = HPG * g + row // DH
        sel = (lane == hid) & (row < _heads_in(g) * DH)
        gcol = jnp.sum(jnp.where(sel, jnp.broadcast_to(gate, (128, 128)), 0.0), axis=1, keepdims=True)
        grep[g] = jnp.broadcast_to(gcol, (128, 128))
        sel8 = (lane8 == HPG * g + row8) & (row8 < _heads_in(g))
        g8 = jnp.sum(jnp.where(sel8, jnp.broadcast_to(gate, (8, 128)), 0.0), axis=1, keepdims=True)
        omg[g] = jnp.broadcast_to(1.0 - g8, (8, 128))
    wr = wr_v[...].reshape(1, D).astype(F32)
    wr = jnp.concatenate([wr, jnp.zeros((1, DP - D), F32)], axis=1)
    wr_col[...] = jnp.broadcast_to(wr, (128, DP)).T

    r128 = _iota((128, 128), 0)
    c128 = _iota((128, 128), 1)
    mrow = _iota((MROWS, 128), 0)
    mlane = _iota((MROWS, 128), 1)
    mhead = jnp.where(mrow < 128, mrow // DH, mrow - 128)
    mmask = (mhead == mlane // DH) & (mlane < HPG * DH) & ((mrow < HPG * DH) | (mrow >= 128))
    ones8 = jnp.ones((8, L), F32)
    kp = 2 * _iota((64, 128), 0)
    qc = _iota((64, 128), 1)
    causal = (jnp.where(kp <= qc, 0x0000FFFF, 0) | jnp.where(kp + 1 <= qc, jnp.int32(-65536), 0))

    def head_window(j):
        return (DH * j // 8) * 8

    def ones_row(j):
        return 0 if DH * j - head_window(j) == 6 else 23

    def ln_in(s):
        rss = []
        for c in range(L // 128):
            cs = slice(128 * c, 128 * (c + 1))
            m, rs = _ln_stats(_pk(x_v[s, :, cs]))
            mh = m.astype(BF16).astype(F32)
            mw = pltpu.bitcast((m - mh).astype(BF16).astype(F32), I32)
            mhw = pltpu.bitcast(mh, I32)
            w0 = mw | lax.shift_right_logical(mhw, 16)
            w1 = lax.shift_right_logical(mhw, 16)
            r8 = _iota((8, 128), 0)
            xe_v[:, cs] = jnp.where(r8 == 0, w0, jnp.where(r8 == 1, w1, 0))
            rss.append(rs)
        return jnp.concatenate(rss, axis=1)

    def proj(i, s):
        xr = _up(jnp.concatenate([_pk(x_v[s]), xe_v[...]], axis=0))
        return lax.dot_general(_up(wT[_blk(i, QV_ROWS // 2), 0:D + 16]), xr,
                               (((1,), (0,)), ((), ())),
                               preferred_element_type=F32)

    def out_proj_post(s):
        for c in range(L // 128):
            cs = slice(128 * c, 128 * (c + 1))
            ot = _up(jnp.concatenate([_unfold(oT, 4 * g + c, 32) for g in range(NG)], axis=0))
            hf = jnp.concatenate(
                [x_v[s, HD * u:HD * (u + 1), cs].astype(F32)
                 + jnp.dot(_up(woT[HD // 2 * u:HD // 2 * (u + 1), :]), ot, preferred_element_type=F32)
                 for u in range(2)], axis=1)
            h_v[_blk(4 * s + c, D // 4), :] = _pk(hf.astype(BF16))
            hw = _unfold(h_v, 4 * s + c + zero, D // 4)
            m, rs = _ln_stats(hw)
            hf = _f32(hw)
            hn = (hf - m) * rs
            h2_v[s, :, cs] = (hf + hn).astype(BF16)
            r = jnp.broadcast_to(jnp.sum(hn * wr_col[0:D, :], axis=0, keepdims=True), (8, 128))
            best = rb_ref[:, cs]
            upd = r > best
            rb_ref[:, cs] = jnp.where(upd, r, best)
            ib_ref[:, cs] = jnp.where(upd, lane8 + (s * L + 128 * c), ib_ref[:, cs])

    def seg_body(s):
        rs = ln_in(s)
        q = proj(0, s) * rs
        qmax = jnp.max(jnp.abs(q))
        qT_g[0:QV_ROWS // 2, :] = _pk((q * QSCALE).astype(BF16))
        pqT_g[0:QV_ROWS // 2, :] = _pk(_phi(q).astype(BF16))
        k = proj(1, s) * rs
        kmax = jnp.max(jnp.abs(k))
        k_g[:, 0:QV_ROWS] = _pk(k.astype(BF16).T)
        pkT_g[0:QV_ROWS // 2, :] = _pk(_phi(k).astype(BF16))
        v = proj(2, s) * rs
        vmax = jnp.max(jnp.abs(v))
        vT_g[0:QV_ROWS, :] = v
        safe = (qmax * kmax * (DH * QSCALE * 1.02) <= SAFE_BOUND) & (vmax <= V_BOUND)

        f0 = jnp.where(s > 0, s - 1, 3) * (FF // 3)
        for g in range(NG):
            for t in range(3 * g, min(3 * g + 3, 12)):
                fc = pl.multiple_of(f0 + 128 * t, 128)
                wdT[pl.ds(pl.multiple_of(fc // 2, 64), 64), 0:D] = _pk(wd_v[:, pl.ds(fc, 128)].T)
            _group(g)

        @pl.when(jnp.logical_not(safe))
        def _():
            _slow_attention()

        @pl.when(s > 0)
        def _():
            o_copy(s - 1).start()

        @pl.when(s == 0)
        def _():
            f_copy(2).wait()

        @pl.when(s + 1 < NSEG)
        def _():
            x_copy(s + 1).wait()
        out_proj_post(s)

    def _group(g):
        nh = _heads_in(g)
        g2 = slice(64 * g, 64 * (g + 1))
        mr = -(-nh * DH // 8) * 8
        mt = MT[g]
        lhs = jnp.concatenate([mt[0:mr] * grep[g, 0:mr], mt[128:MROWS]], axis=0)
        nd = jnp.dot(lhs, _up(pqT_g[g2, :]), preferred_element_type=F32)
        rden = 1.0 / (nd[mr:mr + 8] + 1e-06)
        for r in range(mr // 8):
            lo, hi = 8 * r, 8 * r + 8
            h0, h1 = lo // DH, min((hi - 1) // DH, HPG - 1)
            rd = jnp.broadcast_to(rden[h0:h0 + 1], (8, L))
            if h1 != h0:
                rd = jnp.where(_iota((8, L), 0) + lo < DH * h1, rd,
                               jnp.broadcast_to(rden[h1:h1 + 1], (8, L)))
            am[g, lo:hi, :] = nd[lo:hi] * rd
        lhs = jnp.concatenate([vT_g[128 * g:128 * g + mr, :], ones8], axis=0)
        upd = lax.dot_general(lhs, _up(pkT_g[g2, :]), (((1,), (1,)), ((), ())),
                              preferred_element_type=F32)
        MT[g, 0:mr] = mt[0:mr] + jnp.where(mmask[0:mr], upd[0:mr], 0.0)
        MT[g, 128:MROWS] = mt[128:MROWS] + jnp.where(mmask[128:MROWS], upd[mr:mr + 8], 0.0)

        def qk(qb, slot):
            nk = (qb + 1) * 128
            qt = qT_g[g2, qb * 128:(qb + 1) * 128]
            rr = _iota((64, 128), 0)
            qm = _up(jnp.concatenate(
                [jnp.where((rr >= 9 * j) & (rr < 9 * j + 9), qt, 0)
                 for j in range(nh)], axis=1))
            sc = jnp.dot(_up(k_g[0:nk // 2, 128 * g:128 * (g + 1)]), qm, preferred_element_type=F32)
            p_buf[256 * slot:256 * slot + nk // 2, 0:nh * 128] = _pk(jnp.exp2(sc).astype(BF16))

        def pv(qb, slot):
            nk = (qb + 1) * 128
            vals = []
            for j in range(nh):
                a2 = 128 * g + head_window(j)
                vw = jnp.where(_iota((24, nk), 0) == ones_row(j), 1.0, vT_g[a2:a2 + 24, 0:nk])
                js = slice(j * 128, (j + 1) * 128)
                p0 = 256 * slot
                pw = p_buf[p0 + (nk - 128) // 2:p0 + nk // 2, js] & causal
                if nk > 128:
                    pw = jnp.concatenate([p_buf[p0:p0 + (nk - 128) // 2, js], pw], axis=0)
                acc = jnp.dot(vw, _up(pw), preferred_element_type=F32)
                rd = omg[g, j:j + 1, :] / acc[ones_row(j):ones_row(j) + 1]
                vals.append((acc, jnp.broadcast_to(rd, (8, 128))))
            rows = []
            for r in range(16):
                lo, hi = 8 * r, 8 * r + 8
                h0, h1 = lo // DH, (hi - 1) // DH
                val = am[g, lo:hi, qb * 128:(qb + 1) * 128] if lo < mr else None
                if h0 < nh:
                    a0 = head_window(h0)
                    d = vals[h0][0][lo - a0:hi - a0] * vals[h0][1]
                    if h1 != h0:
                        if h1 < nh:
                            a1 = head_window(h1)
                            d1 = vals[h1][0][lo - a1:hi - a1] * vals[h1][1]
                        else:
                            d1 = jnp.zeros((8, 128), F32)
                        d = jnp.where(row8 + lo < DH * h1, d, d1)
                    val = d if val is None else val + d
                elif val is None:
                    val = jnp.zeros((8, 128), F32)
                rows.append(val)
            oT[_blk(4 * g + qb, 32), :] = _pk(jnp.concatenate(
                [jnp.concatenate(rows[:8], axis=0), jnp.concatenate(rows[8:], axis=0)],
                axis=1).astype(BF16))

        order = (3, 2, 1, 0)
        for i, qb in enumerate(order):
            qk(qb, i % 2)
            if i > 0:
                pv(order[i - 1], (i - 1) % 2)
        pv(order[-1], (len(order) - 1) % 2)

    def _slow_attention():
        def g_body(g, c):
            oslow[...] = am[g]

            def j_body(j, c2):
                a = pl.multiple_of((DH * j // 16) * 16, 16)
                lo = DH * j

                def q_body(qb, c3):
                    q0 = pl.multiple_of(qb * 128, 128)
                    g64 = pl.multiple_of(g * 64, 64)
                    qt = _up(qT_g[pl.ds(g64, 64), pl.ds(q0, 128)])
                    qm = jnp.where((r128 >= lo) & (r128 < lo + DH), qt, jnp.zeros_like(qt))
                    sc = jnp.dot(_up(k_g[:, pl.ds(pl.multiple_of(g * 128, 128), 128)]), qm,
                                 preferred_element_type=F32)
                    ok = _iota((L, 128), 0) <= _iota((L, 128), 1) + q0
                    sc = jnp.where(ok, sc, -jnp.inf)
                    mx = jnp.max(sc, axis=0, keepdims=True)
                    p = jnp.exp2(sc - mx).astype(BF16)
                    vw = vT_g[pl.ds(pl.multiple_of(2 * g64 + a, 16), 32), :]
                    vw = jnp.where(_iota((32, L), 0) == 31, 1.0, vw)
                    acc = jnp.dot(vw, p, preferred_element_type=F32)
                    rr = _iota((32, 128), 0) + a
                    keep = (rr >= lo) & (rr < lo + DH)
                    gj = grep[g, pl.ds(a, 32), :]
                    val = acc * ((1.0 - gj) / acc[31:32])
                    cur = oslow[pl.ds(a, 32), pl.ds(q0, 128)]
                    oslow[pl.ds(a, 32), pl.ds(q0, 128)] = jnp.where(keep, cur + val, cur)
                    return c3
                return lax.fori_loop(0, 4, q_body, c2)
            lax.fori_loop(0, HPG, j_body, 0)
            for qb in range(4):
                qs = slice(128 * qb, 128 * (qb + 1))
                oT[_blk(4 * g + qb, 32), :] = _pk(
                    jnp.concatenate([oslow[0:64, qs], oslow[64:128, qs]], axis=1).astype(BF16))
            return c
        lax.fori_loop(0, NG, g_body, 0)

    zero = ib_s[0]
    x_copy(0).wait()
    lax.fori_loop(0, NSEG, lambda s, c: (seg_body(s), c)[1], 0)

    o_copy(NSEG - 1).start()
    rb = rb_ref[...]
    rmax = jnp.max(rb)
    idx = jnp.min(jnp.where(rb == rmax, ib_ref[...], SEQ))
    idx = jnp.clip(idx, 0, SEQ - 1)
    hw = _unfold(h_v, idx // 128, D // 4)
    m, rs = _ln_stats(hw)
    hf = _up(hw).astype(F32)
    hn = ((hf - m) * rs).astype(BF16)
    hrow = jnp.concatenate([hn, jnp.zeros((DP - D, 128), BF16)], axis=0).T
    pick_r = _iota((128, DP), 0) == (idx % 128)
    xs = jnp.sum(jnp.where(pick_r, hrow.astype(F32), 0.0), axis=0, keepdims=True)
    xs = jnp.broadcast_to(xs[:, 0:D], (16, D)).astype(BF16)
    for i in range(2):
        f_copy(i).wait()
    gt = jnp.dot(xs, wg_v[...], preferred_element_type=F32)[0:8]
    up = jnp.dot(xs, wu_v[...], preferred_element_type=F32)[0:8]
    act = (gt * jax.nn.sigmoid(gt) * up)
    act = jnp.concatenate([act, act], axis=0).astype(BF16)
    y = jnp.dot(act, _up(wdT[0:FF // 2, 0:D]), preferred_element_type=F32)[0:1]
    y = y * jax.nn.sigmoid(jnp.full((1, D), rmax, F32))
    y = jnp.concatenate([y, jnp.zeros((1, DP - D), F32)], axis=1)
    ycol = jnp.broadcast_to(y, (128, DP)).T[0:D]
    hn = hn.astype(F32)
    new = (hf + (hn + ycol).astype(BF16).astype(F32)).astype(BF16)
    old = (hf + hn).astype(BF16)
    patch_v[...] = jnp.where(_iota((D, 128), 1) == (idx % 128), new, old)
    for s in range(NSEG):
        o_copy(s).wait()
    p0 = pl.multiple_of((idx // 128) * 128, 128)
    cp = pltpu.make_async_copy(patch_v, out_hbm.at[:, pl.ds(p0, 128)], sem_p)
    cp.start()
    cp.wait()


@jax.jit
def pallas_sequential_preLN__memory_aug_infini_attn__moe_arch_mod__prompt_kernel(
    A_x: jax.Array,
    A_wq: jax.Array,
    A_wk: jax.Array,
    A_wv: jax.Array,
    A_wo: jax.Array,
    A_beta: jax.Array,
    B_x: jax.Array,
    B_w_r: jax.Array,
    B_w_gate: jax.Array,
    B_w_up: jax.Array,
    B_w_down: jax.Array,
):
    del B_x
    hbm = pl.BlockSpec(memory_space=pltpu.HBM)
    VM = pltpu.VMEM
    outT = pl.pallas_call(
        _kernel,
        out_shape=jax.ShapeDtypeStruct((D, SEQ), BF16),
        in_specs=[hbm] * 10,
        out_specs=hbm,
        scratch_shapes=[
            VM((NSEG, D, L), BF16),
            VM((4, DP, D), BF16),
            VM((3 * QV_ROWS // 2, DP), I32),
            VM((D // 2, DP), I32),
            VM((D, FF), BF16),
            VM((D, FF), BF16),
            VM((D, FF + FF // 3), BF16),
            VM((H,), BF16),
            VM((D,), BF16),
            VM((DP, 128), F32),
            VM((L // 2, DP), I32),
            VM((NG * 64, L), I32),
            VM((NG * 64, L), I32),
            VM((NG * 64, L), I32),
            VM((DP, L), F32),
            VM((L, HPG * 128), I32),
            VM((NG * 4 * 32, 256), I32),
            VM((NG, 128, L), F32),
            VM((NG, MROWS, 128), F32),
            VM((NG, 128, 128), F32),
            VM((NG, 8, 128), F32),
            VM((NSEG * D, 256), I32),
            VM((NSEG, D, L), BF16),
            VM((D, 128), BF16),
            VM((128, L), F32),
            VM((8, L), F32),
            VM((8, L), I32),
            VM((8, L), I32),
            pltpu.SMEM((1,), I32),
            VM(((FF + FF // 3) // 2, DP), I32),
            pltpu.SemaphoreType.DMA((NSEG,)),
            pltpu.SemaphoreType.DMA((4,)),
            pltpu.SemaphoreType.DMA((3,)),
            pltpu.SemaphoreType.DMA((NSEG,)),
            pltpu.SemaphoreType.DMA(()),
            pltpu.SemaphoreType.DMA((2,)),
        ],
        compiler_params=pltpu.CompilerParams(
            vmem_limit_bytes=64 * 1024 * 1024,
            flags={"XLA_TPU_FORCE_LP_LLO_SCHEDULER": True}),
    )(A_x.reshape(SEQ, D).T, A_wq, A_wk, A_wv, A_wo, A_beta, B_w_r,
      B_w_gate, B_w_up, B_w_down.T)
    return outT.T.reshape(1, SEQ, D)
```
